```python
import os as _os
_os.environ.setdefault("JAX_PLATFORMS", "cpu")
import jax
import jax.numpy as jnp

def _softmax(x, axis=-1):
    return jax.nn.softmax(x, axis=axis)
def _gelu(x):
    return jax.nn.gelu(x, approximate=True)
def _silu(x):
    return jax.nn.silu(x)
def _sigmoid(x):
    return jax.nn.sigmoid(x)
def _layernorm(x, axis=-1, eps=1e-5):
    m = jnp.mean(x, axis=axis, keepdims=True)
    v = jnp.var(x, axis=axis, keepdims=True)
    return (x - m) / jnp.sqrt(v + eps)
def _scatter_add(tgt, idx, src, axis=0):
    return tgt.at[idx].add(src)
def _segment_sum(src, seg, n):
    return jax.ops.segment_sum(src, seg, n)
class _Rng:
    def __init__(self, key):
        self._k = key
    def _next(self):
        self._k, sub = jax.random.split(self._k)
        return sub
    def normal(self, shape):
        return jax.random.normal(self._next(), shape, dtype=jnp.bfloat16)
    def randint(self, lo, hi, shape):
        return jax.random.randint(self._next(), shape, lo, hi, dtype=jnp.int32)
    def uniform(self, shape, lo=0.0, hi=1.0):
        return jax.random.uniform(self._next(), shape, jnp.bfloat16, lo, hi)
    def permutation(self, n):
        return jax.random.permutation(self._next(), n)


kernel_name = 'recurrent_scan__softmax_full_mha__glu_gated_glu__prompt'

def setup_inputs():
    _rng = _Rng(jax.random.key(int.from_bytes(__import__("os").urandom(4), "little")))
    _w = (lambda a: (lambda t: t.astype(jnp.bfloat16) if jnp.issubdtype(t.dtype, jnp.floating) else t)(jnp.asarray(a)))
    def _A_setup():
        B, S, D = 1, 2048, 1024
        return {
            "x": _w((lambda *s: _rng.normal(s) * 0.05)(B, S, D)),
            "wqkv": _w((lambda *s: _rng.normal(s) * 0.05)(D, 3 * D)),
            "wo": _w((lambda *s: _rng.normal(s) * 0.05)(D, D)),
        }
    _A_in = _A_setup()

    def _B_setup():
        B, S, D, F = 1, 2048, 1024, 3584
        return {
            "x": _w((lambda *s: _rng.normal(s) * 0.05)(B, S, D)),
            "w_gate": _w((lambda *s: _rng.normal(s) * 0.05)(D, F)),
            "w_up": _w((lambda *s: _rng.normal(s) * 0.05)(D, F)),
            "w_down": _w((lambda *s: _rng.normal(s) * 0.05)(F, D)),
        }
    _B_in = _B_setup()

    return {
        "A_x": _A_in["x"],
        "A_wqkv": _A_in["wqkv"],
        "A_wo": _A_in["wo"],
        "B_x": _B_in["x"],
        "B_w_gate": _B_in["w_gate"],
        "B_w_up": _B_in["w_up"],
        "B_w_down": _B_in["w_down"],
    }

def reference(A_x, A_wqkv, A_wo, B_x, B_w_gate, B_w_up, B_w_down):
    def _A_ref(x, wqkv, wo):
        B, S, D = x.shape
        H = 32; Dh = D // H
        qkv = (lambda x, *d: x.transpose(*d))((x @ wqkv).reshape(B, S, 3, H, Dh), 2, 0, 3, 1, 4)
        q, k, v = qkv[0], qkv[1], qkv[2]
        scale = Dh ** -0.5
        scores = jnp.einsum("bhqd,bhkd->bhqk", q, k) * scale
        p = _softmax(scores, axis=-1)
        o = jnp.einsum("bhqk,bhkd->bhqd", p, v)
        return (lambda x, *d: x.transpose(*d))(o, 0, 2, 1, 3).reshape(B, S, D) @ wo

    def _B_ref(x, w_gate, w_up, w_down):
        g = jnp.einsum("bsd,df->bsf", x, w_gate)
        u = jnp.einsum("bsd,df->bsf", x, w_up)
        h = _sigmoid(g) * u
        return jnp.einsum("bsf,fd->bsd", h, w_down)

    x = A_x
    xn = _layernorm(x, axis=-1)
    s = _A_ref(xn, A_wqkv, A_wo)
    g = _silu(_B_ref(xn, B_w_gate, B_w_up, B_w_down))
    return x + s * g
```

```python
import functools
import math

import jax
import jax.numpy as jnp
from jax import lax
import jax.experimental.pallas as pl
import jax.experimental.pallas.tpu as pltpu

F32 = jnp.float32
BF16 = jnp.bfloat16

S, D, F, H = 2048, 1024, 3584, 32
DH = D // H
T = 128
BQ = 512
HB = BQ // 2
NB = S // BQ
FC = 512
NG = D // T
QSCALE = DH ** -0.5 * math.log2(math.e)

CFG = dict(lag=2, att_w=1.0, tanh=False)


def _dot(a, b):
    return jnp.dot(a, b, preferred_element_type=F32)


def _tree(xs, op):
    xs = list(xs)
    while len(xs) > 1:
        xs = [op(xs[i], xs[i + 1]) if i + 1 < len(xs) else xs[i] for i in range(0, len(xs), 2)]
    return xs[0]


def _lhs_ops(a11, a12, a21, a22):
    return [(a11 + a22), (a21 + a22), a11, a22, (a11 + a12), (a21 - a11), (a12 - a22)]


def _rhs_op(i, b11, b12, b21, b22):
    def comb(p, q, sign):
        p, q = p().astype(F32), q().astype(F32)
        return (p + q if sign > 0 else p - q).astype(BF16)
    if i == 0:
        return comb(b11, b22, 1)
    if i == 1:
        return b11()
    if i == 2:
        return comb(b12, b22, -1)
    if i == 3:
        return comb(b21, b11, -1)
    if i == 4:
        return b22()
    if i == 5:
        return comb(b11, b12, 1)
    return comb(b21, b22, 1)


def _strassen(lhs, b11, b12, b21, b22, top, bot):
    def m(i):
        return _dot(lhs(i), _rhs_op(i, b11, b12, b21, b22))
    m5 = m(4)
    yield
    m3 = m(2)
    c12 = m3 + m5
    yield
    c11 = m(6) - m5
    yield
    m4 = m(3)
    c11 = c11 + m4
    yield
    m1 = m(0)
    c22 = m3 + m1
    top(c11 + m1, c12)
    yield
    m2 = m(1)
    c21 = m2 + m4
    c22 = c22 - m2
    yield
    bot(c21, c22 + m(5))
    yield


def _interleave(*streams):
    order = []
    for k, (_, n, lo, hi) in enumerate(streams):
        order += [(lo + (hi - lo) * (j + 0.5) / n, k) for j in range(n)]
    for _, k in sorted(order):
        next(streams[k][0])
    for g, *_ in streams:
        assert next(g, "done") == "done"


def _chain(*gens):
    for g in gens:
        yield from g


def _sigmoid(x):
    if CFG["tanh"]:
        return 0.5 * jnp.tanh(0.5 * x) + 0.5
    return jax.nn.sigmoid(x)


def _kernel(x_hbm, wqkv_hbm, wo_hbm, wg_hbm, wu_hbm, wd_hbm, out_hbm,
            x_v, wqkv_v, wo_v, wg_v, wu_v, wd_v,
            xa_s, k_s, vt_s, qt_s, o_s, y_s, out_v, x_sem, w_sem, out_sem):

    def x_copy(b):
        return pltpu.make_async_copy(x_hbm.at[pl.ds(b * BQ, BQ)], x_v.at[b], x_sem.at[b])

    def wqkv_copy(j):
        return pltpu.make_async_copy(wqkv_hbm.at[:, pl.ds(j * D, D)], wqkv_v.at[j], w_sem.at[j])

    late = [pltpu.make_async_copy(h, v, w_sem.at[3 + j]) for j, (h, v) in enumerate(
        ((wg_hbm, wg_v), (wu_hbm, wu_v), (wd_hbm, wd_v), (wo_hbm, wo_v)))]

    def out_copy(b):
        return pltpu.make_async_copy(out_v.at[b], out_hbm.at[pl.ds(b * BQ, BQ)], out_sem.at[b])

    def layernorm(b, rows=32):
        def norm(r):
            x = x_v[b, r:r + rows, :].astype(F32)
            xc = x - jnp.mean(x, axis=-1, keepdims=True)
            var = jnp.mean(xc * xc, axis=-1, keepdims=True)
            return xc * lax.rsqrt(var + 1e-5)
        for r in range(0, HB, rows):
            t, u = norm(r), norm(HB + r)
            ops = _lhs_ops(t[:, :D // 2], t[:, D // 2:], u[:, :D // 2], u[:, D // 2:])
            for i, a in enumerate(ops):
                xa_s[b, i, r:r + rows, :] = a.astype(BF16)
            yield

    def project(b, w1, w2, top, bot):
        lo, hi = slice(0, D // 2), slice(D // 2, D)
        return _strassen(lambda i: xa_s[b, i], lambda: w1(lo), lambda: w2(lo),
                         lambda: w1(hi), lambda: w2(hi), top, bot)

    def qkv_proj(b, j, store):
        for g in range(0, NG, 2):
            def put(half, g=g):
                def f(c1, c2):
                    store(g, half, c1)
                    store(g + 1, half, c2)
                return f
            yield from project(b, lambda r, g=g: wqkv_v[j, r, g * T:(g + 1) * T],
                               lambda r, g=g: wqkv_v[j, r, (g + 1) * T:(g + 2) * T], put(0), put(1))

    def k_proj(b):
        def store(g, half, c):
            k_s[g, pl.ds(pl.multiple_of(b * BQ + half * HB, HB), HB), :] = c.astype(BF16)
        return qkv_proj(b, 1, store)

    def v_proj(b):
        def store(g, half, c):
            vt_s[g, b, :, half * HB:(half + 1) * HB] = c.T.astype(BF16)
        return qkv_proj(b, 2, store)

    def q_proj(b):
        def store(g, half, c):
            qt_s[b, g, :, half * HB:(half + 1) * HB] = (c * QSCALE).T.astype(BF16)
        return qkv_proj(b, 0, store)

    NC = S // T

    def attention(b, g):
        pend, outs, acc = [], [], [None]

        def pv(j, c, p, alpha, l):
            kb, kc = divmod(c * T, BQ)
            a = _dot(vt_s[g, kb, j * DH:(j + 1) * DH, kc:kc + T], p)
            if c > 0:
                a = (acc[0].reshape(DH // 8, 8, BQ) * alpha[None]).reshape(DH, BQ) + a
            acc[0] = a
            if c == NC - 1:
                outs.append(a / jnp.sum(l, axis=0, keepdims=True))
                if j == T // DH - 1:
                    o_s[b % 2, g] = jnp.concatenate(outs, axis=0).T

        for j in range(T // DH):
            m = l = None
            for c in range(NC):
                q = qt_s[b, g, j * DH:(j + 1) * DH, :]
                if j:
                    q = jnp.concatenate([jnp.zeros((j * DH, BQ), BF16), q], axis=0)
                s = _dot(k_s[g, c * T:(c + 1) * T, :(j + 1) * DH], q).reshape(T // 8, 8, BQ)
                mc = _tree([s[i] for i in range(T // 8)], jnp.maximum)
                mc = jnp.broadcast_to(jnp.max(mc, axis=0, keepdims=True), (8, BQ))
                alpha = None
                if c == 0:
                    m = mc
                else:
                    mn = jnp.maximum(m, mc)
                    alpha = jnp.exp2(m - mn)
                    m = mn
                p = jnp.exp2(s - m[None])
                lc = _tree([p[i] for i in range(T // 8)], jnp.add)
                l = lc if c == 0 else l * alpha + lc
                pend.append((j, c, p.reshape(T, BQ).astype(BF16), alpha, l))
                if len(pend) > CFG["lag"]:
                    pv(*pend.pop(0))
                yield
        while pend:
            pv(*pend.pop(0))
            yield

    n_att = (T // DH) * NC + CFG["lag"]

    def ffn(b, f):
        f0 = pl.multiple_of(f * FC, FC)
        h = {}
        for t in range(FC // T):
            def put(half, t=t):
                def fn(gate, up):
                    h[half, t] = _sigmoid(gate) * up
                return fn
            yield from project(b, lambda r, t=t: wg_v[r, pl.ds(f0 + t * T, T)],
                               lambda r, t=t: wu_v[r, pl.ds(f0 + t * T, T)], put(0), put(1))
            if t % 2:
                h[t // 2] = [a.astype(BF16) for a in _lhs_ops(h[0, t - 1], h[0, t], h[1, t - 1], h[1, t])]
        def w(k, n):
            return lambda: jnp.concatenate(
                [wd_v[pl.ds(f0 + (2 * u + k) * T, T), n:n + 2 * T] for u in range(FC // T // 2)], axis=0)
        for i in range(7):
            a = jnp.concatenate([h[u][i] for u in range(FC // T // 2)], axis=1)
            for n in range(0, D // 2, 2 * T):
                y_s[i, :, n:n + 2 * T] += _dot(a, _rhs_op(i, w(0, n), w(0, D // 2 + n), w(1, n), w(1, D // 2 + n)))
                yield

    n_ffn = 7 * (FC // T) + 14

    def finish(b):
        def o(half, k):
            return jnp.concatenate(
                [o_s[b % 2, k * NG // 2 + u, half * HB:(half + 1) * HB, :] for u in range(NG // 2)], axis=1)
        ops = [a.astype(BF16) for a in _lhs_ops(o(0, 0), o(0, 1), o(1, 0), o(1, 1))]
        lo, hi = slice(0, D // 2), slice(D // 2, D)
        for n in range(0, D // 2, T):
            n1, n2 = slice(n, n + T), slice(D // 2 + n, D // 2 + n + T)
            m = lambda i, n1=n1: y_s[i, :, n1]
            def put(rows, cols, s, y):
                out_v[b, rows, cols] = (x_v[b, rows, cols].astype(F32) + s * (y * _sigmoid(y))).astype(BF16)
            def top(s1, s2, n1=n1, n2=n2, m=m):
                put(slice(0, HB), n1, s1, m(0) + m(3) - m(4) + m(6))
                put(slice(0, HB), n2, s2, m(2) + m(4))
            def bot(s1, s2, n1=n1, n2=n2, m=m):
                put(slice(HB, BQ), n1, s1, m(1) + m(3))
                put(slice(HB, BQ), n2, s2, m(0) - m(1) + m(2) + m(5))
            yield from _strassen(lambda i: ops[i], lambda: wo_v[lo, n1], lambda: wo_v[lo, n2],
                                 lambda: wo_v[hi, n1], lambda: wo_v[hi, n2], top, bot)
        out_copy(b).start()

    n_proj = 7 * NG // 2

    x_copy(0).start()
    wqkv_copy(1).start()
    x_copy(0).wait()
    x_copy(1).start()
    _interleave((layernorm(0), HB // 32, 0, 1))
    wqkv_copy(1).wait()
    for b in range(2, NB):
        x_copy(b).start()
    wqkv_copy(2).start()
    wqkv_copy(0).start()

    def k_step(b, _):
        x_copy(b + 1).wait()
        _interleave((k_proj(b), n_proj, 0, 1), (layernorm(b + 1), HB // 32, 0, 1))
    lax.fori_loop(0, NB - 1, k_step, None)
    for c in late:
        c.start()
    _interleave((k_proj(NB - 1), n_proj, 0, 1))
    wqkv_copy(2).wait()
    wqkv_copy(0).wait()

    def vq_step(b, _):
        _interleave((_chain(v_proj(b), q_proj(b)), 2 * n_proj, 0, 1))
    lax.fori_loop(0, NB, vq_step, None)
    for c in late:
        c.wait()

    def block(b, _):
        @pl.when(b == 0)
        def _():
            _interleave((attention(b, 0), n_att, 0, 1))

        @pl.when(b > 0)
        def _():
            _interleave((attention(b, 0), n_att, 0, 0.97), (finish(b - 1), n_proj, 0, 1))

        y_s[...] = jnp.zeros(y_s.shape, F32)

        def step(f, _):
            _interleave((attention(b, f + 1), n_att, 0, CFG["att_w"]), (ffn(b, f), n_ffn, 0, 1))
        lax.fori_loop(0, F // FC, step, None)
    lax.fori_loop(0, NB, block, None)
    _interleave((finish(NB - 1), n_proj, 0, 1))
    for b in range(NB):
        out_copy(b).wait()


@jax.jit
def pallas_recurrent_scan__softmax_full_mha__glu_gated_glu__prompt_kernel(
        A_x, A_wqkv, A_wo, B_x, B_w_gate, B_w_up, B_w_down):
    del B_x
    any_spec = pl.BlockSpec(memory_space=pl.ANY)
    out = pl.pallas_call(
        _kernel,
        out_shape=jax.ShapeDtypeStruct((S, D), BF16),
        in_specs=[any_spec] * 6,
        out_specs=any_spec,
        scratch_shapes=[
            pltpu.VMEM((NB, BQ, D), BF16),
            pltpu.VMEM((3, D, D), BF16),
            pltpu.VMEM((D, D), BF16),
            pltpu.VMEM((D, F), BF16),
            pltpu.VMEM((D, F), BF16),
            pltpu.VMEM((F, D), BF16),
            pltpu.VMEM((NB, 7, HB, D // 2), BF16),
            pltpu.VMEM((NG, S, T), BF16),
            pltpu.VMEM((NG, NB, T, BQ), BF16),
            pltpu.VMEM((NB, NG, T, BQ), BF16),
            pltpu.VMEM((2, NG, BQ, T), F32),
            pltpu.VMEM((7, HB, D // 2), F32),
            pltpu.VMEM((NB, BQ, D), BF16),
            pltpu.SemaphoreType.DMA((NB,)),
            pltpu.SemaphoreType.DMA((7,)),
            pltpu.SemaphoreType.DMA((NB,)),
        ],
        compiler_params=pltpu.CompilerParams(vmem_limit_bytes=120 * 2 ** 20),
        name="fused_block",
    )(A_x.reshape(S, D), A_wqkv, A_wo, B_w_gate, B_w_up, B_w_down)
    return out.reshape(A_x.shape)
```

```python
import contextlib
import math

import jax
import numpy as np
import jax.numpy as jnp
from jax import lax
import jax.experimental.pallas as pl
import jax.experimental.pallas.tpu as pltpu

F32 = jnp.float32
BF16 = jnp.bfloat16
U32 = jnp.uint32

S, D, F, H = 2048, 1024, 3584, 32
DH = D // H
T = 128
BQ = 512
NB = S // BQ
NG = D // T
QR = BQ // 4
NF = F // (4 * T)
QSCALE = DH ** -0.5 * math.log2(math.e)

CFG = dict(dord=(4, 8, 0, 11, 3, 14, 6, 20, 17, 23), qshare=16, vhk=1, xp=0, hparts=((0,), (1,), (2,), (3,), (4,), (5,), (6,)), hsteps=68, pk=3, pvfirst=0, rs=1, rm=1, lag=2, scopes=False, gpi=3, only=None, ln_rows=32, ktmp=1, dtmp=0, x0=2, h_hi=(7,) * 5, oh_hi=(7,) * 5, split=1, atie=3,
           kb=2, ln_rows2=16, parts=((1, 5), (3,), (4, 6), (2,), (0,)),
           st=((0,), (1,), (2,)), waits={0: "k0 s1", 1: "k1 t3", 2: "k2 x1 s2", 3: "k3 s3", 4: "x2", 6: "x3"},
           plan={2: (1, 2), 4: (2, 2), 6: (3, 2)})


def scope(n):
    return jax.named_scope(n) if CFG["scopes"] else contextlib.nullcontext()


def _dot(a, b):
    return jnp.dot(a, b, preferred_element_type=F32)


def _tree(xs, op):
    xs = list(xs)
    while len(xs) > 1:
        xs = [op(xs[i], xs[i + 1]) if i + 1 < len(xs) else xs[i] for i in range(0, len(xs), 2)]
    return xs[0]


def _force(g):
    if isinstance(g, tuple):
        return tuple(_force(a) for a in g)
    return g() if callable(g) else g


def _add(p, q):
    if isinstance(p, tuple):
        return tuple(_add(a, b) for a, b in zip(p, q))
    return _force(p).astype(F32) + _force(q).astype(F32)


def _sub(p, q):
    if isinstance(p, tuple):
        return tuple(_sub(a, b) for a, b in zip(p, q))
    return _force(p).astype(F32) - _force(q).astype(F32)


def _grid(levels, block, r=0, c=0):
    if levels == 0:
        return lambda: block(r, c)
    return tuple(tuple(_grid(levels - 1, block, 2 * r + i, 2 * c + j) for j in range(2)) for i in range(2))


def _leaves(g, r=0, c=0):
    if isinstance(g, tuple):
        for i in range(2):
            for j in range(2):
                yield from _leaves(g[i][j], 2 * r + i, 2 * c + j)
    else:
        yield r, c, g


def _lhs_op(i, a):
    (a11, a12), (a21, a22) = a
    if i in (2, 3):
        return a11 if i == 2 else a22
    op, p, q = {0: (_add, a11, a22), 1: (_add, a21, a22), 4: (_add, a11, a12),
                5: (_sub, a21, a11), 6: (_sub, a12, a22)}[i]
    return op(p, q)


def _rhs_op(i, b):
    (b11, b12), (b21, b22) = b
    if i in (1, 4):
        return b11 if i == 1 else b22
    op, p, q = {0: (_add, b11, b22), 2: (_sub, b12, b22), 3: (_sub, b21, b11),
                5: (_add, b11, b12), 6: (_add, b21, b22)}[i]
    return op(p, q)


def _lhs_ops(a):
    if not isinstance(a, tuple):
        return [_force(a)]
    return [op for i in range(7) for op in _lhs_ops(_lhs_op(i, a))]


def _rows(ref, ix, r, n):
    return jnp.stack([ref[(*ix, pl.ds(r + k, n // 2, stride=2), slice(None))] for k in range(2)])


def _pack(v):
    return pltpu.pack_elementwise([v[0], v[1]], packed_dtype=BF16)


def _park(refs, g):
    if refs is None:
        return g
    def put(ref, v):
        ix = (slice(0, v.shape[0]), slice(0, v.shape[1]))
        ref[ix] = v
        return lambda: ref[ix]
    if isinstance(g, tuple):
        return tuple(tuple(put(refs[2 * r + c], g[r][c]) for c in range(2)) for r in range(2))
    return put(refs, g)


def _tie(w, zeros):
    if not zeros:
        return w
    n = w.shape[0] // 8
    at = {((u + 1) * n) // len(zeros) - 1: pltpu.bitcast(z, U32) for u, z in enumerate(zeros)}
    head = jnp.concatenate([w[8 * r:8 * r + 8, :T] | at[r] if r in at else w[8 * r:8 * r + 8, :T]
                            for r in range(n)], axis=0)
    return jnp.concatenate([head, w[:, T:]], axis=1) if w.shape[1] > T else head


def _spread(*phases):
    for work, steps in phases:
        for k in range(steps):
            yield [job() for job in work[k * len(work) // steps:(k + 1) * len(work) // steps]]
    while True:
        yield []


def _strassen(lhs, b, emit, tmp, side, idx=0):
    def m(i):
        rhs = _rhs_op(i, b)
        if not isinstance(rhs, tuple):
            a = _tie(lhs(7 * idx + i), next(side) if side else None)
            return _dot(pltpu.bitcast(a, BF16), _force(rhs).astype(BF16))
        c = {}
        _strassen(lhs, rhs, lambda r, s, v: c.__setitem__((r, s), v), tmp[1:], side, 7 * idx + i)
        return ((c[0, 0], c[0, 1]), (c[1, 0], c[1, 1]))
    t = tmp[0]() if tmp[0] else [None] * 5
    m2 = _park(t[0], m(1))
    m4 = m(3)
    emit(1, 0, _add(m2, m4))
    m4 = _park(t[1], m4)
    m5 = _park(t[2], m(4))
    m3 = m(2)
    emit(0, 1, _add(m3, m5))
    t22 = _park(t[3], _sub(m3, m2))
    m1 = _park(t[4], m(0))
    emit(0, 0, _add(_sub(_add(m(6), m1), m5), m4))
    emit(1, 1, _add(_add(m(5), m1), t22))


def _matmul(lhs, w, emit, tmp, side=None):
    def emit_grid(i, j, g):
        for r, c, v in _leaves(g, i, j):
            emit(r, c, v)
    _strassen(lhs, _grid(len(tmp), w), emit_grid, tmp, side)


def _hopcroft_kerr():
    u = np.array([[1, 0], [0, 1], [-1, -1]])
    v = np.array([[0, -1], [1, 0], [-1, 1]])
    e = np.eye(4, dtype=int)
    prods = []
    def dot(r, c, p, q):
        prods.extend([(np.outer(r, u[p]), np.outer(c, v[q])), (np.outer(r, u[q]), np.outer(c, v[p]))])
    kind = (1, 0, 2, 1)
    for i in range(4):
        dot(e[i], e[i], (kind[i] + 1) % 3, (kind[i] + 2) % 3)
    def pair(ra, ca, s, rb, cb, t):
        prods.append((np.outer(ra, u[t]) + np.outer(rb, u[s]), np.outer(ca, v[t]) - np.outer(cb, v[s])))
        dot(rb - ra, cb + ca, t, s)
    for i, j in ((0, 1), (0, 2), (1, 2), (1, 3), (2, 3)):
        pair(e[i], e[i], kind[i], e[j], e[j], kind[j])
    pair(e[1] - e[0], e[1] + e[0], 2, e[3], e[3], kind[3])
    return prods


def _combine(terms):
    pos = [g for k, g in terms if k > 0]
    neg = [g for k, g in terms if k < 0]
    if not pos:
        return -1, _tree(neg, _add)
    return 1, _sub(_tree(pos, _add), _tree(neg, _add)) if neg else _tree(pos, _add)


def _hk_operand(coef, block):
    return _combine([(k, block(i, j)) for (i, j), k in np.ndenumerate(coef) if k])


def _hk_lhs_ops(a):
    block = lambda r, k: _grid(1, lambda u, q: a(r, 2 * k + q, u))
    return [op for coef, _ in _hopcroft_kerr() for op in _lhs_ops(_hk_operand(coef, block)[1])]


def _matmul_hk(lhs, w, emit, slots, inner, side=None):
    prods = _hopcroft_kerr()
    slots = iter(slots)
    p = {}
    def park(sign, v):
        return sign, _park(next(slots), v)
    def m(i):
        ca, cb = prods[i]
        sign, rhs = _hk_operand(cb, lambda c, k: _grid(1, lambda q, u: w(2 * k + q, c, u)))
        c = {}
        _strassen(lhs, rhs, lambda r, s, v: c.__setitem__((r, s), v), [inner], side, i)
        v = jnp.concatenate([jnp.concatenate([c[r, 0], c[r, 1]], axis=1) for r in range(2)], axis=0)
        return sign * (1 if (ca > 0).any() else -1), v
    def total(*terms):
        sign, v = terms[0][0] * terms[0][1][0], terms[0][1][1]
        for k, (s, g) in terms[1:]:
            if k * s == sign:
                v = _add(v, g)
            elif sign > 0:
                v = _sub(v, g)
            else:
                sign, v = 1, _sub(g, v)
        return sign, v
    def out(r, c, *terms):
        sign, v = total(*terms)
        emit(r, c, v if sign > 0 else -v)
        return sign, v
    for i in CFG["dord"]:
        p[i] = park(*m(i))
    def diag(i, k):
        v = m(k)
        out(i, i, (1 - 2 * (k % 2), v), (2 * (k % 2) - 1, p[k ^ 1]))
        p[k] = park(*v)
    diag(1, 2)
    p10 = m(10)
    out(0, 1, (1, p10), (-1, p[8]), (-1, p[0]), (1, p[2]))
    p10 = park(*p10)
    diag(0, 1)
    p9 = m(9)
    out(1, 0, (1, p9), (-1, p[8]), (-1, p[1]), (1, p[3]))
    p9 = park(*p9)
    diag(3, 7)
    y13 = out(1, 3, (-1, m(19)), (1, p[17]), (1, p[3]), (-1, p[7]))
    t03 = park(*total((1, y13), (-1, p[6]), (1, p9)))
    y31 = out(3, 1, (-1, m(18)), (1, p[17]), (1, p[2]), (-1, p[6]))
    t30 = park(*total((-1, y31), (1, p[7]), (-1, p10)))
    out(0, 3, (-1, m(25)), (1, p[23]), (1, t03))
    out(3, 0, (1, m(24)), (-1, p[23]), (1, t30))
    diag(2, 5)
    out(0, 2, (-1, m(13)), (1, p[11]), (1, p[1]), (-1, p[5]))
    out(2, 0, (-1, m(12)), (1, p[11]), (1, p[0]), (-1, p[4]))
    out(2, 1, (1, m(15)), (-1, p[14]), (-1, p[3]), (1, p[5]))
    out(1, 2, (1, m(16)), (-1, p[14]), (-1, p[2]), (1, p[4]))
    out(2, 3, (1, m(22)), (-1, p[20]), (-1, p[4]), (1, p[6]))
    out(3, 2, (1, m(21)), (-1, p[20]), (-1, p[5]), (1, p[7]))


def put(ref, ix, r, cols, v):
    v = v.astype(BF16)
    if ref.dtype == U32:
        v, r = pltpu.bitcast(v, U32), r // 2
    ref[(*ix, slice(r, r + v.shape[0]), cols)] = v


def get(ref, ix, r, n, cols):
    if ref.dtype == U32:
        return pltpu.bitcast(ref[(*ix, slice(r // 2, (r + n) // 2), cols)], BF16)
    return ref[(*ix, slice(r, r + n), cols)]


def _sigmoid(x):
    return 0.5 * jnp.tanh(0.5 * x) + 0.5


def _kernel(x_hbm, wqkv_hbm, wo_hbm, wg_hbm, wu_hbm, wd_hbm, out_hbm,
            x_v, wo_v, wgu_v, wd_v, xb_s, h_s, t1_s, t2_s, z_s, x_sem, wk_sem, w_sem, gu_sem, out_sem):
    only = CFG["only"]
    X0 = CFG["x0"]
    count = [0]

    def inner():
        count[0] += 1
        k = 5 * (count[0] % (len(t1_s) // 5))
        return t1_s[k:k + 5]

    def outer():
        return [t2_s[4 * k:4 * k + 4] for k in range(5)]

    def keep(ref):
        v = ref[(z_s[0],) + (0,) * (len(ref.shape) - 3) + (slice(0, 16), slice(0, T))]
        x_v[0, 0:16, 0:T] = (pltpu.bitcast(v, F32) if v.dtype == U32 else v).astype(BF16)
        c = pltpu.make_async_copy(x_v.at[0], out_hbm.at[pl.ds(0, BQ)], out_sem.at[0])
        c.start(); c.wait()

    def x_copy(b):
        return pltpu.make_async_copy(x_hbm.at[pl.ds(b * BQ, BQ)], x_v.at[b], x_sem.at[b])

    def x0_copy(u):
        rows = pl.ds(u * BQ // X0, BQ // X0)
        return pltpu.make_async_copy(x_hbm.at[rows], x_v.at[0, rows], x_sem.at[NB + u])

    def gu_copies(f):
        cols = pl.ds(pl.multiple_of(f * 4 * T, 4 * T), 4 * T)
        return [pltpu.make_async_copy(w.at[:, cols], wgu_v.at[f % 2, j], gu_sem.at[f % 2, j])
                for j, w in enumerate((wg_hbm, wu_hbm))]

    wo_copy = pltpu.make_async_copy(wo_hbm, wo_v, w_sem.at[2])
    wd_copies = [pltpu.make_async_copy(wd_hbm.at[:, pl.ds(n * D // 2, D // 2)], wd_v.at[n], w_sem.at[3 + n]) for n in range(2)]

    def attention_phase(xa_s, wk_v, wqv_v, xn_s, k_s, qv_s, p_s, acc_s):
        def wk_copy(j):
            return pltpu.make_async_copy(wqkv_hbm.at[:, pl.ds(D + j * 2 * T, 2 * T)], wk_v[j], wk_sem.at[j])

        def wqv_copy(j):
            return pltpu.make_async_copy(wqkv_hbm.at[:, pl.ds(2 * j * D, D)], wqv_v.at[j], w_sem.at[j])

        for c in [x0_copy(u) for u in range(X0)] + [wk_copy(j) for j in CFG["st"][0]]:
            c.start()

        @pl.loop(0, 2)
        def _(i):
            z_s[i] = 0
        for ref in t1_s + t2_s:
            ref[pl.ds(pl.multiple_of(z_s[0], 8), 8), 0:T] = jnp.zeros((8, T), F32)
        for ref in xn_s:
            ref[NG + z_s[0], 0:8] = jnp.zeros((8, T), F32)
        xa_s[z_s[0], 0:8, 0:T] = jnp.zeros((8, T), U32)
        for ref in xb_s:
            ref[7, 0:8, 0:T] = jnp.zeros((8, T), U32)
        h_s[0, 0, 0, S // 4:, :] = jnp.zeros((8, T), F32)

        def layernorm(b, r, rows, z):
            x = x_v[b, r:r + rows, :].astype(F32)
            xc = x - jnp.mean(x, axis=-1, keepdims=True)
            var = jnp.mean(xc * xc, axis=-1, keepdims=True)
            xn = xc * lax.rsqrt(var + 1e-5)
            for t in range(NG):
                xn_s[b][t + z, r:r + rows, :] = xn[:, t * T:(t + 1) * T]

        def ln_jobs(b):
            rows = CFG["ln_rows2"]
            z0, z1 = z_s[0], z_s[1]
            def job(r):
                layernorm(b, r, rows, z0)
                return xn_s[b][NG + z1, 0:8, :]
            return [lambda r=r: job(r) for r in range(0, BQ, rows)]

        KB = CFG["kb"]

        def k_first(b, j, side, ops):
            def emit(r, c, v):
                put(k_s, (2 * j + c,), b * BQ + r * BQ // 2, slice(None), v)
            _matmul(lambda i: ops[i], lambda r, c: wk_v[j][r * D // 2:(r + 1) * D // 2, c * T:(c + 1) * T],
                    emit, [inner if CFG["ktmp"] else None], side)

        def make_operands(lo, hi):
            ops = _lhs_ops(_grid(2, lambda r, c: jnp.concatenate([jnp.concatenate(
                [_rows(xn_s[b], (2 * c + u,), r * QR, QR) for u in range(2)], axis=2)
                for b in range(lo, hi)], axis=1)))
            def make(i):
                xa_s[i, lo * QR // 2:hi * QR // 2, :] = _pack(ops[i])
            return make

        def k_rest():
            make = make_operands(KB, NB)
            def lhs(i):
                make(i)
                return xa_s[i, KB * QR // 2:, :]
            def emit(r, c, v):
                for b in range(KB, NB):
                    for u in range(2):
                        put(k_s, (2 * c + u,), b * BQ + r * QR, slice(None),
                            v[(b - KB) * QR:(b - KB + 1) * QR, u * T:(u + 1) * T])
            _matmul(lhs, lambda r, c: wk_v[c][r * D // 4:(r + 1) * D // 4, :], emit, [outer, inner])

        def qv_proj(j):
            make = make_operands(0, KB) if j == 0 else (lambda i: None)
            def lhs(i):
                make(i)
                return xa_s[i]
            def emit(r, c, v):
                if j == 0:
                    v = v * QSCALE
                for b in range(NB):
                    for u in range(2):
                        put(qv_s, (j, 2 * c + u, b), 0, slice(r * QR, (r + 1) * QR),
                            v[b * QR:(b + 1) * QR, u * T:(u + 1) * T].T)
            order = CFG["dord"] + (2, 10, 1, 9, 7, 19, 18, 25, 24, 5, 13, 12, 15, 16, 22, 21)
            n = CFG["qshare"]
            if j == 0 or not CFG["vhk"]:
                _matmul(lhs, lambda r, c: wqv_v[j, r * D // 4:(r + 1) * D // 4, c * D // 4:(c + 1) * D // 4],
                        emit, [outer, inner], _spread((xb_jobs(order[n:] if j else order[:n]), 48)))
                return
            _matmul_hk(lambda i: xb_s[i // 7][i % 7],
                       lambda r, c, u: wqv_v[j, r * D // 4:(r + 1) * D // 4, (2 * c + u) * T:(2 * c + u + 1) * T],
                       emit, t2_s, inner, _spread((xb_jobs(order[n:]), 70)))

        def xb_jobs(which):
            z0, z1 = z_s[0], z_s[1]
            prods = _hopcroft_kerr()
            def job(i, row, t):
                block = lambda r, k: _grid(1, lambda u, q: _rows(
                    xn_s[2 * u + row // QR], (2 * (2 * k + q) + t,), r * QR + row % QR, 16))
                for j, v in enumerate(_lhs_ops(_hk_operand(prods[i][0], block)[1])):
                    xb_s[i][j + z0, row // 2:row // 2 + 8, t * T:(t + 1) * T] = _pack(v)
                return xb_s[i][7 + z1, 0:8, 0:T]
            return [lambda i=i, row=row, t=t: job(i, row, t)
                    for row in range(0, 2 * QR, 16) for t in range(2) for i in which]

        NC = S // T
        NJ = T // DH
        lag, gpi = CFG["lag"], CFG["gpi"]

        ties = []

        def pv(acc, b, g, j, c, p, alpha, l):
            kb, kc = divmod(c * T, BQ)
            a = _dot(get(qv_s, (1, g, kb), j * DH, DH, slice(kc, kc + T)), p)
            if c > 0:
                a = (acc.reshape(DH // 8, 8, BQ) * alpha[None]).reshape(DH, BQ) + a
            if c == NC - 1:
                acc_s[j * DH:(j + 1) * DH] = a / jnp.sum(l, axis=0, keepdims=True)
                if j == NJ - 1:
                    for r in range(4):
                        h_s[g % 2, r, g // 2, pl.ds(pl.multiple_of(b * QR, QR), QR), :] = acc_s[0:T, r * QR:(r + 1) * QR].T
                    ties.append(h_s[z_s[1], 0, 0, S // 4:, :])
            return a

        def carried(job):
            l = acc_s[T + DH:T + DH + 8]
            return acc_s[T:T + DH], [
                (job % NB, job // NB, NJ - 1, NC - lag + u, p_s[u], acc_s[T + DH + 8 * (u + 1):T + DH + 8 * (u + 2)], l)
                for u in range(lag)]

        def att_jobs(first, n, start=False):
            acc, pend = (None, []) if start else carried(first - 1)
            for u in range(n):
                b, g = (first + u) % NB, (first + u) // NB
                for j in range(NJ):
                    m = l = None
                    for c in range(NC):
                        if CFG["pvfirst"]:
                            acc = pv(acc, *pend.pop(0))
                        q = get(qv_s, (0, g, b), j * DH, DH, slice(None))
                        if j:
                            q = jnp.concatenate([jnp.zeros((j * DH, BQ), BF16), q], axis=0)
                        k = k_s[g, c * T // 2:(c + 1) * T // 2, :]
                        if c == lag + CFG["atie"] and ties:
                            k = _tie(k, [ties.pop()])
                        s = _dot(pltpu.bitcast(k, BF16)[:, :(j + 1) * DH], q).reshape(T // 8, 8, BQ)
                        mn = s[0] if c == 0 else jnp.maximum(m, s[0])
                        if CFG["rm"] == 1:
                            for t in range(1, T // 8):
                                mn = jnp.maximum(mn, s[t])
                        else:
                            mn = jnp.maximum(mn, s[1])
                            for t in range(2, T // 8, 2):
                                mn = jnp.maximum(mn, jnp.maximum(s[t], s[t + 1]))
                        mn = jnp.broadcast_to(jnp.max(mn, axis=0, keepdims=True), (8, BQ))
                        alpha = None if c == 0 else jnp.exp2(m - mn)
                        m = mn
                        p = jnp.exp2(s - m[None])
                        if CFG["rs"] == 0:
                            lc = _tree([p[t] for t in range(T // 8)], jnp.add)
                            l = lc if c == 0 else l * alpha + lc
                        elif CFG["rs"] == 1:
                            l = None if c == 0 else l * alpha
                            for t in range(T // 8 - 2, -1, -2):
                                l = p[t] + p[t + 1] if l is None else l + (p[t] + p[t + 1])
                        else:
                            l = None if c == 0 else l * alpha
                            for t in range(T // 8 - 4, -1, -4):
                                lc = (p[t] + p[t + 1]) + (p[t + 2] + p[t + 3])
                                l = lc if l is None else l + lc
                        pend.append((b, g, j, c, p.reshape(T, BQ).astype(BF16), alpha, l))
                        if len(pend) > lag:
                            acc = pv(acc, *pend.pop(0))
            acc_s[T:T + DH] = acc
            acc_s[T + DH:T + DH + 8] = pend[-1][6]
            for u in range(lag):
                p_s[u] = pend[u][4]
                acc_s[T + DH + 8 * (u + 1):T + DH + 8 * (u + 2)] = pend[u][5]

        run_k = only in (None, "k")
        with scope("z_pro"):
            for u in range(X0):
                with scope("z_wx0" + str(u)):
                    x0_copy(u).wait()
                for j in CFG["st"][u + 1]:
                    wk_copy(j).start()
                if run_k:
                    for r in range(u * BQ // X0, (u + 1) * BQ // X0, CFG["ln_rows"]):
                        layernorm(0, r, CFG["ln_rows"], 0)
        with scope("z_k"):
            side = None
            for b in range(KB):
                for j in range(NG // 2):
                    for w in CFG["waits"].get(4 * b + j, "").split():
                        if w[0] in "st":
                            (x_copy if w[0] == "s" else wk_copy)(int(w[1])).start()
                            continue
                        with scope("z_w" + w):
                            (wk_copy if w[0] == "k" else x_copy)(int(w[1])).wait()
                        if w == "x2":
                            wqv_copy(0).start()
                    if j == 0:
                        ops = [_pack(v) for v in _lhs_ops(_grid(1, lambda r, c: jnp.concatenate(
                            [_rows(xn_s[b], (4 * c + u,), r * BQ // 2, BQ // 2) for u in range(4)], axis=2)))]
                    if 4 * b + j in CFG["plan"]:
                        nb, n = CFG["plan"][4 * b + j]
                        side = _spread((ln_jobs(nb), 7 * n))
                    if run_k:
                        k_first(b, j, side, ops)
        with scope("z_k2"):
            wqv_copy(0).wait()
            wqv_copy(1).start()
            wo_copy.start()
            if only in (None, "k2", "k"):
                k_rest()
        with scope("z_qv"):
            if only in (None, "q"):
                qv_proj(0)
        with scope("z_v"):
            wqv_copy(1).wait()
            if only in (None, "v"):
                qv_proj(1)
        with scope("z_att"):
            wo_copy.wait()
            for c in wd_copies + gu_copies(0):
                c.start()
            if only in (None, "att", "k"):
                head = NB * NG % gpi
                att_jobs(0, head, True)
                lax.fori_loop(0, NB * NG // gpi, lambda i, _: att_jobs(head + i * gpi, gpi), None)
                acc, pend = carried(NB * NG - 1)
                for job in pend:
                    acc = pv(acc, *job)
        if only is not None:
            for ref in [qv_s, xa_s, k_s, h_s] + xn_s:
                keep(ref)

    pl.run_scoped(
        attention_phase,
        pltpu.VMEM((49, S // 8, D // 4), U32),
        [pltpu.VMEM((D, 2 * T), BF16)] * (NG // 2),
        pltpu.VMEM((2, D, D), BF16),
        [pltpu.VMEM((NG + 1, BQ, T), F32)] * NB,
        pltpu.VMEM((NG, S // 2, T), U32) if CFG["pk"] & 1 else pltpu.VMEM((NG, S, T), BF16),
        pltpu.VMEM((2, NG, NB, T // 2, BQ), U32) if CFG["pk"] & 2 else pltpu.VMEM((2, NG, NB, T, BQ), BF16),
        pltpu.VMEM((CFG["lag"], T, BQ), BF16),
        pltpu.VMEM((T + DH + 8 * (CFG["lag"] + 1), BQ), F32),
    )
    for c in wd_copies:
        c.wait()

    def ffn_phase(ha_s, out_v):
        ZERO = 7 * NF
        for ref in ha_s:
            ref[ZERO, 0:8] = jnp.zeros((8, T), U32)

        def h_operands(f):
            z1 = z_s[1]
            def job(r, part):
                a = _grid(2, lambda i, j: _rows(h_s, (0, i, j), r, 16))
                for i in part:
                    for j, v in enumerate(_lhs_ops(_lhs_op(i, a))):
                        ha_s[i][7 * f + j, r // 2:r // 2 + 8, :] = _pack(v)
                return _tree([ha_s[i][ZERO + z1, 0:8, :] for i in part], jnp.bitwise_or)
            if CFG.get("pmaj"):
                return [lambda r=r, p=p: job(r, p) for p in CFG["hparts"] for r in range(0, S // 4, 16)]
            return [lambda r=r, p=p: job(r, p) for r in range(0, S // 4, 16) for p in CFG["hparts"]]

        def gate_up(f, _):
            for c in gu_copies(f):
                c.wait()

            @pl.when(f + 1 < NF)
            def _():
                for c in gu_copies(f + 1):
                    c.start()
            def emit(r, c, v):
                h_s[0, r, c, :S // 4] = _sigmoid(v[:, :T]) * v[:, T:]
            _matmul_hk(lambda i: xb_s[i // 7][i % 7],
                       lambda r, c, u: wgu_v[f % 2, u, r * D // 4:(r + 1) * D // 4, c * T:(c + 1) * T],
                       emit, t2_s, inner, _spread((h_operands(f), CFG["hsteps"])))
        with scope("z_gu"):
            if only in (None, "gu"):
                lax.fori_loop(0, NF, gate_up, None)
            else:
                for c in gu_copies(0):
                    c.wait()

        def out_proj():
            ops = _lhs_ops(_grid(2, lambda r, c: _rows(h_s, (1, r, c), 0, S // 4)))
            def emit(r, c, v):
                for b in range(NB):
                    out_v[b // 2, c // 2, (b % 2) * BQ + r * QR:(b % 2) * BQ + (r + 1) * QR,
                          (c % 2) * 2 * T:(c % 2 + 1) * 2 * T] = v[b * QR:(b + 1) * QR].astype(BF16)
            _matmul(lambda i: jnp.concatenate([pre[i](), _pack(ops[i])], axis=1),
                    lambda r, c: wo_v[r * D // 4:(r + 1) * D // 4, c * D // 4:(c + 1) * D // 4],
                    emit, [outer, inner], _spread(*zip(h_operands2(), CFG["oh_hi"])))
        pre = [lambda i=i: ha_s[i // 7][i % 7] for i in range(49)]

        def h_operands2():
            z0, z1 = z_s[0], z_s[1]
            def job(r, part):
                a = _grid(2, lambda i, j: _rows(h_s, (0, i, j), r, 16))
                for i in part:
                    for j, v in enumerate(_lhs_ops(_lhs_op(i, a))):
                        xb_s[i][j + z0, r % 256 // 2:r % 256 // 2 + 8, (r // 256) * T:(r // 256 + 1) * T] = _pack(v)
                return _tree([xb_s[i][7 + z1, 0:8, 0:T] for i in part], jnp.bitwise_or)
            return [[lambda r=r, p=p: job(r, p) for r in range(0, S // 4, 16)] for p in CFG["parts"]]

        with scope("z_op"):
            if only in (None, "op"):
                out_proj()

        def out_copies(it, last):
            half, n = it // 2, it % 2
            hb, hc = BQ // 2, D // 4
            parts = [(b * BQ + hb, hc, hc) for b in range(2)] if last else (
                [(b * BQ, 0, 2 * hc) for b in range(2)] + [(b * BQ + hb, 0, hc) for b in range(2)])
            return [pltpu.make_async_copy(
                out_v.at[half, n, pl.ds(r, hb), pl.ds(c, w)],
                out_hbm.at[pl.ds(pl.multiple_of(half * (S // 2) + r, hb), hb), pl.ds(pl.multiple_of(n * (D // 2) + c, hc), w)],
                out_sem.at[0]) for r, c, w in parts]

        def down(it, _, split=CFG['split'] == 1):
            half, n = it // 2, it % 2
            rows = pl.ds(pl.multiple_of(half * QR, QR), QR)
            if CFG["xp"] & 1:
                rows = pl.ds(0, QR)
            if CFG["xp"] & 2:
                n = 0
            if CFG["xp"] & 4:
                half = 0
            col = lambda c: pl.ds(pl.multiple_of((4 * n + c) * T, T), T)
            def emit(r, c, y):
                g = y * _sigmoid(y)
                for b in range(2):
                    ix = (half, n, slice(b * BQ + r * QR, b * BQ + (r + 1) * QR), slice(c * T, (c + 1) * T))
                    x = x_v[2 * half + b, r * QR:(r + 1) * QR, col(c)].astype(F32)
                    out_v[ix] = (x + out_v[ix].astype(F32) * g[b * QR:(b + 1) * QR]).astype(BF16)
                if (r, c) == (1, 1) and split:
                    for cp in out_copies(it, False):
                        cp.start()
            _matmul(
                lambda i: jnp.concatenate([ha_s[i // 7][7 * f + i % 7, rows, :] for f in range(1, NF)] + [xb_s[i // 7][i % 7, :, pl.ds(pl.multiple_of(half * T, T), T)]], axis=1),
                lambda r, c: jnp.concatenate([wd_v[n, (4 * f + r) * T:(4 * f + r + 1) * T, c * T:(c + 1) * T] for f in range(NF)], axis=0),
                emit, [outer if CFG["dtmp"] & 2 else None, inner if CFG["dtmp"] & 1 else None])
            for cp in ([] if split else out_copies(it, False)) + out_copies(it, True):
                cp.start()
        with scope("z_dn"):
            if only in (None, "dn"):
                lax.fori_loop(0, 3 if CFG["split"] == 2 else 4, down, None)
                if CFG["split"] == 2:
                    down(3, None, True)
        with scope("z_tail"):
            if only in (None, "dn"):
                for it in range(4):
                    for cp in out_copies(it, False) + out_copies(it, True):
                        cp.wait()
        if only is not None:
            for ref in ha_s + xb_s + [out_v, h_s]:
                keep(ref)

    pl.run_scoped(
        ffn_phase,
        [pltpu.VMEM((7 * NF + 1, S // 8, T), U32)] * 7,
        pltpu.VMEM((2, 2, S // 2, D // 2), BF16),
    )


@jax.jit
def pallas_recurrent_scan__softmax_full_mha__glu_gated_glu__prompt_kernel(
        A_x, A_wqkv, A_wo, B_x, B_w_gate, B_w_up, B_w_down):
    del B_x
    any_spec = pl.BlockSpec(memory_space=pl.ANY)
    out = pl.pallas_call(
        _kernel,
        out_shape=jax.ShapeDtypeStruct((S, D), BF16),
        in_specs=[any_spec] * 6,
        out_specs=any_spec,
        scratch_shapes=[
            pltpu.VMEM((NB, BQ, D), BF16),
            pltpu.VMEM((D, D), BF16),
            pltpu.VMEM((2, 2, D, 4 * T), BF16),
            pltpu.VMEM((2, F, D // 2), BF16),
            [pltpu.VMEM((8, S // 16, D // 4), U32)] * 26,
            pltpu.VMEM((2, 4, 4, S // 4 + 8, T), F32),
            [pltpu.VMEM((S // 4, D // 4), F32)] * 10,
            [pltpu.VMEM((S // 4, D // 4), F32)] * 20,
            pltpu.SMEM((2,), jnp.int32),
            pltpu.SemaphoreType.DMA((NB + 4,)),
            pltpu.SemaphoreType.DMA((4,)),
            pltpu.SemaphoreType.DMA((5,)),
            pltpu.SemaphoreType.DMA((2, 2)),
            pltpu.SemaphoreType.DMA((4,)),
        ],
        compiler_params=pltpu.CompilerParams(vmem_limit_bytes=126 * 2 ** 20, flags=CFG.get("flags")),
        name=CFG.get("name", "fused_block"),
    )(A_x.reshape(S, D), A_wqkv, A_wo, B_w_gate, B_w_up, B_w_down)
    return out.reshape(A_x.shape)
```

```python
import math

import jax
import jax.numpy as jnp
import numpy as np
from jax import lax
import jax.experimental.pallas as pl
import jax.experimental.pallas.tpu as pltpu

F32 = jnp.float32
BF16 = jnp.bfloat16
U32 = jnp.uint32

S, D, F, H = 2048, 1024, 3584, 32
DH = D // H
T = 128
BQ = 512
NB = S // BQ
NG = D // T
NC = S // T
NF = F // (4 * T)
NV = 16
KB = 2
QSCALE = DH ** -0.5 * math.log2(math.e)
SUM_RANGE = 2.0 ** 60


def _dot(a, b):
    return jnp.dot(a, b, preferred_element_type=F32)


def _bits(v):
    return pltpu.bitcast(v, U32)


def _words(ref, *ix):
    return ref.bitcast(U32)[ix]


def _tree(xs, op):
    xs = list(xs)
    while len(xs) > 1:
        xs = [op(xs[i], xs[i + 1]) if i + 1 < len(xs) else xs[i] for i in range(0, len(xs), 2)]
    return xs[0]


def _tie(w, zeros):
    if not zeros:
        return w
    n = w.shape[0] // 8
    at = {((u + 1) * n) // len(zeros) - 1: _bits(z) for u, z in enumerate(zeros)}
    head = jnp.concatenate([w[8 * r:8 * r + 8, :T] | at[r] if r in at else w[8 * r:8 * r + 8, :T]
                            for r in range(n)], axis=0)
    return jnp.concatenate([head, w[:, T:]], axis=1) if w.shape[1] > T else head


def _spread(*phases):
    for jobs, steps in phases:
        for k in range(steps):
            yield [job() for job in jobs[k * len(jobs) // steps:(k + 1) * len(jobs) // steps]]
    while True:
        yield []


def _force(g):
    return g() if callable(g) else g


def _add(p, q):
    if isinstance(p, tuple):
        return tuple(_add(a, b) for a, b in zip(p, q))
    return _force(p).astype(F32) + _force(q).astype(F32)


def _sub(p, q):
    if isinstance(p, tuple):
        return tuple(_sub(a, b) for a, b in zip(p, q))
    return _force(p).astype(F32) - _force(q).astype(F32)


def _grid(levels, block, r=0, c=0):
    if levels == 0:
        return lambda: block(r, c)
    return tuple(tuple(_grid(levels - 1, block, 2 * r + i, 2 * c + j) for j in range(2)) for i in range(2))


def _leaves(g, r=0, c=0):
    if isinstance(g, tuple):
        for i in range(2):
            for j in range(2):
                yield from _leaves(g[i][j], 2 * r + i, 2 * c + j)
    else:
        yield r, c, g


def _park(refs, g):
    if refs is None:
        return g
    if isinstance(g, tuple):
        return tuple(tuple(_park(refs[2 * r + c], g[r][c]) for c in range(2)) for r in range(2))
    ix = (slice(0, g.shape[0]), slice(0, g.shape[1]))
    refs[ix] = g
    return lambda: refs[ix]


def _lhs_op(i, a):
    (a11, a12), (a21, a22) = a
    if i in (2, 3):
        return a11 if i == 2 else a22
    op, p, q = {0: (_add, a11, a22), 1: (_add, a21, a22), 4: (_add, a11, a12),
                5: (_sub, a21, a11), 6: (_sub, a12, a22)}[i]
    return op(p, q)


def _rhs_op(i, b):
    (b11, b12), (b21, b22) = b
    if i in (1, 4):
        return b11 if i == 1 else b22
    op, p, q = {0: (_add, b11, b22), 2: (_sub, b12, b22), 3: (_sub, b21, b11),
                5: (_add, b11, b12), 6: (_add, b21, b22)}[i]
    return op(p, q)


def _lhs_ops(a):
    if not isinstance(a, tuple):
        return [_force(a)]
    return [op for i in range(7) for op in _lhs_ops(_lhs_op(i, a))]


def _strassen(lhs, b, emit, tmp, side, idx=0):
    def m(i):
        rhs = _rhs_op(i, b)
        if isinstance(rhs, tuple):
            c = {}
            _strassen(lhs, rhs, lambda r, s, v: c.update({(r, s): v}), tmp[1:], side, 7 * idx + i)
            return ((c[0, 0], c[0, 1]), (c[1, 0], c[1, 1]))
        a, *more = lhs(7 * idx + i)
        a = pltpu.bitcast(_tie(a, next(side)), BF16)
        return _dot(jnp.concatenate([a] + more, axis=1) if more else a, _force(rhs).astype(BF16))
    t = tmp[0]()
    m2 = _park(t[0], m(1))
    m4 = m(3)
    emit(1, 0, _add(m2, m4))
    m4 = _park(t[1], m4)
    m5 = _park(t[2], m(4))
    m3 = m(2)
    emit(0, 1, _add(m3, m5))
    t22 = _park(t[3], _sub(m3, m2))
    m1 = _park(t[4], m(0))
    emit(0, 0, _add(_sub(_add(m(6), m1), m5), m4))
    emit(1, 1, _add(_add(m(5), m1), t22))


def _matmul(lhs, w, emit, tmp, side):
    def emit_grid(i, j, g):
        for r, c, v in _leaves(g, i, j):
            emit(r, c, v)
    _strassen(lhs, _grid(len(tmp), w), emit_grid, tmp, side)


def _hopcroft_kerr():
    u = np.array([[1, 0], [0, 1], [-1, -1]])
    v = np.array([[0, -1], [1, 0], [-1, 1]])
    e = np.eye(4, dtype=int)
    kind = (1, 0, 2, 1)
    prods = []

    def inner(r, c, p, q):
        prods.extend([(np.outer(r, u[p]), np.outer(c, v[q])), (np.outer(r, u[q]), np.outer(c, v[p]))])

    def pair(ra, ca, s, rb, cb, t):
        prods.append((np.outer(ra, u[t]) + np.outer(rb, u[s]), np.outer(ca, v[t]) - np.outer(cb, v[s])))
        inner(rb - ra, cb + ca, t, s)
    for i in range(4):
        inner(e[i], e[i], (kind[i] + 1) % 3, (kind[i] + 2) % 3)
    for i, j in ((0, 1), (0, 2), (1, 2), (1, 3), (2, 3)):
        pair(e[i], e[i], kind[i], e[j], e[j], kind[j])
    pair(e[1] - e[0], e[1] + e[0], 2, e[3], e[3], kind[3])
    return prods


HK = _hopcroft_kerr()
HK_ORDER = (4, 8, 0, 11, 3, 14, 6, 20, 17, 23, 2, 10, 1, 9, 7, 19, 18, 25, 24, 5, 13, 12, 15, 16, 22, 21)


def _hk_operand(coef, block):
    pos = [block(i, k) for (i, k), c in np.ndenumerate(coef) if c > 0]
    neg = [block(i, k) for (i, k), c in np.ndenumerate(coef) if c < 0]
    if not pos:
        return -1, _tree(neg, _add)
    return 1, _sub(_tree(pos, _add), _tree(neg, _add)) if neg else _tree(pos, _add)


def _matmul_hk(lhs, w, emit, slots, inner, side):
    slots = iter(slots)

    def m(i):
        sign, rhs = _hk_operand(HK[i][1], lambda c, k: _grid(1, lambda q, u: w(2 * k + q, c, u)))
        c = {}
        _strassen(lhs, rhs, lambda r, s, v: c.update({(r, s): v}), [inner], side, i)
        v = jnp.concatenate([jnp.concatenate([c[r, 0], c[r, 1]], axis=1) for r in range(2)], axis=0)
        return sign * (1 if (HK[i][0] > 0).any() else -1), v

    def park(sign, v):
        return sign, _park(next(slots), v)

    def total(*terms):
        sign, v = terms[0][0] * terms[0][1][0], terms[0][1][1]
        for k, (s, g) in terms[1:]:
            if k * s == sign:
                v = _add(v, g)
            elif sign > 0:
                v = _sub(v, g)
            else:
                sign, v = 1, _sub(g, v)
        return sign, v

    def out(r, c, *terms):
        sign, v = total(*terms)
        emit(r, c, v if sign > 0 else -v)
        return sign, v

    def diagonal(k):
        v = m(k)
        out(k // 2, k // 2, (1 - 2 * (k % 2), v), (2 * (k % 2) - 1, p[k ^ 1]))
        p[k] = park(*v)

    p = {i: park(*m(i)) for i in HK_ORDER[:10]}
    diagonal(2)
    p10 = m(10)
    out(0, 1, (1, p10), (-1, p[8]), (-1, p[0]), (1, p[2]))
    p10 = park(*p10)
    diagonal(1)
    p9 = m(9)
    out(1, 0, (1, p9), (-1, p[8]), (-1, p[1]), (1, p[3]))
    p9 = park(*p9)
    diagonal(7)
    y13 = out(1, 3, (-1, m(19)), (1, p[17]), (1, p[3]), (-1, p[7]))
    t03 = park(*total((1, y13), (-1, p[6]), (1, p9)))
    y31 = out(3, 1, (-1, m(18)), (1, p[17]), (1, p[2]), (-1, p[6]))
    t30 = park(*total((-1, y31), (1, p[7]), (-1, p10)))
    out(0, 3, (-1, m(25)), (1, p[23]), (1, t03))
    out(3, 0, (1, m(24)), (-1, p[23]), (1, t30))
    diagonal(5)
    out(0, 2, (-1, m(13)), (1, p[11]), (1, p[1]), (-1, p[5]))
    out(2, 0, (-1, m(12)), (1, p[11]), (1, p[0]), (-1, p[4]))
    out(2, 1, (1, m(15)), (-1, p[14]), (-1, p[3]), (1, p[5]))
    out(1, 2, (1, m(16)), (-1, p[14]), (-1, p[2]), (1, p[4]))
    out(2, 3, (1, m(22)), (-1, p[20]), (-1, p[4]), (1, p[6]))
    out(3, 2, (1, m(21)), (-1, p[20]), (-1, p[5]), (1, p[7]))


def _kernel(x_hbm, wqkv_hbm, wo_hbm, wg_hbm, wu_hbm, wd_hbm, out_hbm,
            x_v, wgu_v, xb_s, h_s, t1_s, t2_s, z_s, x_sem, wk_sem, w_sem, gu_sem, out_sem):
    turn = [0]

    def inner():
        turn[0] ^= 5
        return t1_s[turn[0]:turn[0] + 5]

    def outer():
        return [t2_s[4 * k:4 * k + 4] for k in range(5)]

    def xb(i):
        return jnp.concatenate([_words(xb_s[i // 7], i % 7, t) for t in range(2)], axis=1),

    def gu_copies(f):
        cols = pl.ds(pl.multiple_of(f * 4 * T, 4 * T), 4 * T)
        return [pltpu.make_async_copy(w.at[:, cols], wgu_v.at[f & 1, j], gu_sem.at[f & 1, j])
                for j, w in enumerate((wg_hbm, wu_hbm))]

    def attention_phase(wk_v, wqv_v, xn_s, xa_s, k_s, q_s, v_s, kh_s, kb_s, qf_s, kv_s, ot_s, p_s, acc_s):
        n = BQ // 2
        x_in = [pltpu.make_async_copy(x_hbm.at[pl.ds(i * n, n)], x_v.at[i // 2, pl.ds(i % 2 * n, n)], x_sem.at[i])
                for i in range(2 * NB)]
        wk_in = [pltpu.make_async_copy(wqkv_hbm.at[:, pl.ds(D + j * 2 * T, 2 * T)], wk_v[j], wk_sem.at[j])
                 for j in range(NG // 2)]
        wqv_in = [pltpu.make_async_copy(wqkv_hbm.at[:, pl.ds(2 * j * D, D)], wqv_v.at[j], w_sem.at[j])
                  for j in range(2)]

        def layernorm(b, r, rows, z):
            x = x_v[b, r:r + rows, :].astype(F32)
            xc = x - jnp.mean(x, axis=-1, keepdims=True)
            xn = xc * lax.rsqrt(jnp.mean(xc * xc, axis=-1, keepdims=True) + 1e-5)
            for t in range(NG):
                xn_s[b][t + z, r:r + rows, :] = xn[:, t * T:(t + 1) * T]

        def layernorm_jobs(b):
            z0, z1 = z_s[0], z_s[1]

            def job(r):
                layernorm(b, r, 16, z0)
                return xn_s[b][NG + z1, 0:8, :]
            return [lambda r=r: job(r) for r in range(0, BQ, 16)]

        def xa(lo, hi, first):
            ops = [_lhs_ops(_grid(2, lambda r, c, t=t: jnp.concatenate(
                [xn_s[b][2 * c + t, r * T:(r + 1) * T, :] for b in range(lo, hi)], axis=0))) for t in range(2)]

            def lhs(i):
                for t in range(2):
                    xa_s[i, t, lo * T:hi * T] = ops[t][i].astype(BF16)
                return jnp.concatenate([_words(xa_s, i, t, slice(first * T // 2, None)) for t in range(2)], axis=1),
            return lhs

        def xb_jobs(which):
            z0, z1 = z_s[0], z_s[1]

            def block(t, z):
                return lambda r, k: _grid(1, lambda u, q: jnp.concatenate(
                    [xn_s[b][z + 2 * (2 * k + q) + t, r * T:(r + 1) * T, :] for b in (2 * u, 2 * u + 1)], axis=0))
            ops = {(i, t): jnp.stack(_lhs_ops(_hk_operand(HK[i][0], block(t, z_s[n]))[1]))
                   for n, i in enumerate(which) for t in range(2)}

            def job(i, row, t):
                xb_s[i][pl.ds(z0, 7), t, row:row + 16, :] = ops[i, t][:, row:row + 16].astype(BF16)
                return _words(xb_s[i], 7 + z1, 0, slice(0, 8))
            return [lambda i=i, row=row, t=t: job(i, row, t)
                    for row in range(0, 2 * T, 16) for t in range(2) for i in which]

        def emit_k(r, c, v):
            for b in range(KB, NB):
                for u in range(2):
                    k_s[2 * c + u, b * BQ + r * T:b * BQ + (r + 1) * T, :] = (
                        v[(b - KB) * T:(b - KB + 1) * T, u * T:(u + 1) * T].astype(BF16))

        def emit_transposed(ref, r, c, v):
            for b in range(NB):
                for u in range(2):
                    heads = slice(4 * (2 * c + u), 4 * (2 * c + u + 1))
                    ref[heads, 4 * b + r] = v[b * T:(b + 1) * T, u * T:(u + 1) * T].T.reshape(4, DH, T).astype(BF16)

        def tiles(ref, h, b):
            return jnp.concatenate([_words(ref, h, 4 * b + t) for t in range(4)], axis=1)

        def to_lane0(k, h):
            return pltpu.roll(k, (T - DH * (h & 3)) & (T - 1), 1)

        def head_jobs(h, slot, after=lambda v: v):
            z0, z1 = z_s[0], z_s[1]

            def pick():
                kv = jnp.concatenate([_words(k_s, h >> 2, slice(r - NV // 2, r)) for r in range(T, S // 2 + 1, T)], axis=0)
                kv_s[z0, :DH] = pltpu.bitcast(to_lane0(after(kv), h), BF16).astype(F32).T[:DH]
                return kv_s[z1, DH:DH + 8]

            def queries(b):
                qf_s[slot][z0, b] = pltpu.bitcast(after(tiles(q_s, h, b)), BF16).astype(F32).reshape(DH // 8, 8, BQ)
                return qf_s[slot][z1, NB, 0, :, 0:T]

            def move(r):
                kh_s[slot][z0, r:r + T, :] = to_lane0(after(_words(k_s, h >> 2, slice(r, r + T))), h)
                return kh_s[slot][z1, S // 2:S // 2 + 8, :]

            def splat(d):
                kb_s[slot][z0, d] = after(jnp.broadcast_to(kv_s[0, d:d + 1, :], (T, T))).T
                return kb_s[slot][z1, DH, 0:8, :]
            return ([pick] + [lambda b=b: queries(b) for b in range(NB)]
                    + [lambda r=r: move(r) for r in range(0, S // 2, T)] + [lambda d=d: splat(d) for d in range(DH)])

        def output_jobs(g, b, after=lambda v: v):
            z1 = z_s[1]

            def job(r):
                h_s[g & 1, r, g >> 1, pl.ds(pl.multiple_of(b * T, T), T), :] = after(ot_s[g & 1, b, :, r * T:(r + 1) * T]).T
                return h_s[z1, 0, 0, S // 4:S // 4 + 8, :]
            return [lambda r=r: job(r) for r in range(4)]

        def put_head(h, b, o):
            ot_s[(h >> 2) & 1, b, pl.ds(pl.multiple_of((h & 3) * DH, DH), DH), :] = o

        def pv(ties, acc, h, b, c, p, l):
            a = _dot(pltpu.bitcast(_words(v_s, h + z_s[b], c), BF16), p)
            if c > 0:
                a = acc + a
            if c == NC - 1:
                l = jnp.sum(l, axis=0, keepdims=True)
                r = pltpu.reciprocal(l, approx=True)
                r = r * (2.0 - l * r)
                o = a * r
                put_head(h, b, o)
                ot_s[2 + z_s[0], 0, 8:16, :] += _tree([o[t:t + 8] for t in range(0, DH, 8)], jnp.add) * 0.0 + (l + r)
                ties.append(ot_s[2 + z_s[1], 0, 0:8, 0:T])
            return a

        def attention(h, slot):
            acc, pend = acc_s[:DH], [((h + H - 1) & (H - 1), NB - 1, NC - 1, p_s[...], acc_s[DH:])]
            zero = jnp.tile(_bits(h_s[z_s[1], 0, 0, S // 4:S // 4 + 8, :]), (NV // 8, 1))
            now, ties = [None], []

            def after(v):
                z = jnp.tile(_bits(now[0]) & zero[:8], (1, v.shape[1] // T))
                return jnp.concatenate([pltpu.bitcast(_bits(v[:8]) | z, v.dtype), v[8:]], axis=0)

            def vector_scores(b, e):
                cols = []
                for t in range(BQ // T):
                    z = z_s[e]
                    q = jnp.stack([jnp.broadcast_to(qf_s[slot][z, b, :, i:i + 1, t * T:(t + 1) * T], (DH // 8, NV, T))
                                   for i in range(8)], axis=1).reshape(DH, NV, T)
                    v = kb_s[slot][z_s[4 * b + t], :DH, e * NV:(e + 1) * NV, :] * q
                    if cols:
                        first = pltpu.bitcast(_bits(v[0]) | (_bits(cols[-1]) & zero), F32)
                        v = jnp.concatenate([first[None], v[1:]], axis=0)
                    cols.append(jnp.sum(v, axis=0))
                return jnp.concatenate(cols, axis=1)

            side = _spread(([], 2),
                           (output_jobs(((h >> 2) + NG - 1) & (NG - 1), h & 3, after), 4),
                           (head_jobs(jnp.minimum(h + 1, H - 1), 1 - slot, after), 55))
            late = [[]] * 3
            for b in range(NB):
                l = None
                for c in range(NC):
                    nv = NV if c % 2 and (b, c) != (0, 1) else 0
                    late.append(next(side))
                    k = _tie(kh_s[slot][z_s[b], c * T // 2:((c + 1) * T - nv) // 2, :],
                             late.pop(0) + ([ties.pop()] if c == 3 else []))
                    s = _dot(pltpu.bitcast(k, BF16)[:, :DH], pltpu.bitcast(tiles(q_s, h + z_s[c], b), BF16))
                    now[0] = s[96:104, :T]
                    if nv:
                        s = jnp.concatenate([s, vector_scores(b, c // 2)], axis=0)
                    p = jnp.exp2(s)
                    for t in range(0, T, 16):
                        two = p[t:t + 8] + p[t + 8:t + 16]
                        l = two if l is None else l + two
                    pend.append((h, b, c, p.astype(BF16), l))
                    if len(pend) > 2:
                        acc = pv(ties, acc, *pend.pop(0))
            acc_s[:DH] = pv(ties, acc, *pend.pop(0))
            p_s[...], acc_s[DH:] = pend[0][3:]

        def exact_attention(job, _):
            h, b = job >> 2, job & 3
            q = pltpu.bitcast(tiles(q_s, h, b), BF16)

            def step(i, carry):
                m, l, acc = carry
                k = to_lane0(_words(k_s, h >> 2, pl.ds(pl.multiple_of(i * (BQ // 2), BQ // 2), BQ // 2)), h)
                s = _dot(pltpu.bitcast(k, BF16)[:, :DH], q)
                top = jnp.maximum(m, jnp.max(s, axis=0, keepdims=True))
                alpha, p = jnp.exp2(m - top), jnp.exp2(s - top)
                return (top, l * alpha + jnp.sum(p, axis=0, keepdims=True),
                        acc * alpha + _dot(pltpu.bitcast(tiles(v_s, h, i), BF16), p.astype(BF16)))
            _, l, acc = lax.fori_loop(0, NB, step, (jnp.full((1, BQ), -jnp.inf, F32), jnp.zeros((1, BQ), F32),
                                                    jnp.zeros((DH, BQ), F32)))
            put_head(h, b, acc / l)

            @pl.when((h & 3) == 3)
            def _():
                for run in output_jobs(h >> 2, b):
                    run()

        for c in x_in[:2] + wk_in[:1]:
            c.start()

        @pl.loop(0, z_s.shape[0])
        def _(i):
            z_s[i] = 0
        for ref in t1_s + t2_s:
            ref[pl.ds(pl.multiple_of(z_s[0], 8), 8), 0:T] = jnp.zeros((8, T), F32)
        for ref in xn_s:
            ref[NG + z_s[0], 0:8] = jnp.zeros((8, T), F32)
        xa_s[z_s[0], 0, 0:16] = jnp.zeros((16, T), BF16)
        for ref in xb_s:
            ref[7, 0, 0:16] = jnp.zeros((16, T), BF16)
        for slot in range(2):
            kh_s[slot][0, S // 2:S // 2 + 8, :] = jnp.zeros((8, T), U32)
            qf_s[slot][0, NB, 0, :, 0:T] = jnp.zeros((8, T), F32)
            kb_s[slot][0, DH, 0:8, :] = jnp.zeros((8, T), F32)
        h_s[0, 0, 0, S // 4:S // 4 + 8, :] = jnp.zeros((8, T), F32)
        kv_s[0, DH:DH + 8] = jnp.zeros((8, T), F32)
        ot_s[1] = jnp.zeros((NB, T, BQ), F32)
        ot_s[2, 0, 0:16] = jnp.zeros((16, BQ), F32)
        p_s[...] = jnp.zeros(p_s.shape, BF16)
        acc_s[...] = jnp.ones(acc_s.shape, F32)

        for i in range(2):
            x_in[i].wait()
            wk_in[i + 1].start()
            for r in range(i * n, (i + 1) * n, 32):
                layernorm(0, r, 32, 0)
        traffic = {0: ([wk_in[0]], [x_in[2]]), 1: ([wk_in[1]], [wk_in[3], x_in[3]]),
                   2: ([wk_in[2], x_in[2]], [x_in[4]]), 3: ([wk_in[3], x_in[3]], x_in[5:7]),
                   4: (x_in[4:6], [wqv_in[0], x_in[7]]), 6: (x_in[6:8], [])}
        side = _spread()
        for step in range(KB * NG // 2):
            b, j = divmod(step, NG // 2)
            wait, start = traffic.get(step, ([], []))
            for c in wait:
                c.wait()
            for c in start:
                c.start()
            if j == 0:
                ops = [(_bits(v[:, :T].astype(BF16)), v[:, T:].astype(BF16)) for v in _lhs_ops(_grid(
                    1, lambda r, c: jnp.concatenate([xn_s[b][4 * c + t, r * n:(r + 1) * n, :] for t in range(4)], axis=1)))]
            if step == 2:
                jobs = layernorm_jobs(1)
                side = _spread(([], 1), (jobs[:16], 6), ([], 1), (jobs[16:], 6))
            if step in (4, 6):
                side = _spread(([], 1), (layernorm_jobs(step // 2), 13))

            def emit(r, c, v):
                k_s[2 * j + c, b * BQ + r * n:b * BQ + (r + 1) * n, :] = v.astype(BF16)
            _matmul(lambda i: ops[i], lambda r, c: wk_v[j][r * D // 2:(r + 1) * D // 2, c * T:(c + 1) * T],
                    emit, [inner], side)

        wqv_in[0].wait()
        for c in wqv_in[1:] + gu_copies(0):
            c.start()
        _matmul(xa(KB, NB, KB), lambda r, c: wk_v[c][r * D // 4:(r + 1) * D // 4, :], emit_k, [outer, inner], _spread())
        _matmul(xa(0, KB, 0), lambda r, c: wqv_v[0, r * D // 4:(r + 1) * D // 4, c * D // 4:(c + 1) * D // 4],
                lambda r, c, v: emit_transposed(q_s, r, c, v * QSCALE), [outer, inner],
                _spread((xb_jobs(HK_ORDER[:16]), 48)))
        wqv_in[1].wait()
        _matmul_hk(xb, lambda r, c, u: wqv_v[1, r * D // 4:(r + 1) * D // 4, (2 * c + u) * T:(2 * c + u + 1) * T],
                   lambda r, c, v: emit_transposed(v_s, r, c, v), t2_s, inner,
                   _spread((xb_jobs(HK_ORDER[16:]), 70), (head_jobs(0, 0), 100)))
        for c in gu_copies(0):
            c.wait()

        @pl.loop(0, H // 2)
        def _(i):
            attention(2 * i, 0)
            pl.when(z_s[0] == 0)(lambda: attention(2 * i + 1, 1))

        for b in range(NB):
            if b == NB - 1:
                pv([], acc_s[:DH], H - 1, b, NC - 1, p_s[...], acc_s[DH:])
            for run in output_jobs(NG - 1, b):
                run()

        @pl.when(jnp.max(jnp.where(ot_s[2, 0, 8:16, :] <= SUM_RANGE, 0, 1)) > 0)
        def _():
            lax.fori_loop(0, H * NB, exact_attention, None)

    pl.run_scoped(
        attention_phase,
        [pltpu.VMEM((D, 2 * T), BF16)] * (NG // 2),
        pltpu.VMEM((2, D, D), BF16),
        [pltpu.VMEM((NG + 1, BQ, T), F32)] * NB,
        pltpu.VMEM((49, 2, S // 4, T), BF16),
        pltpu.VMEM((NG, S, T), BF16),
        pltpu.VMEM((H, NC, DH, T), BF16),
        pltpu.VMEM((H, NC, DH, T), BF16),
        [pltpu.VMEM((1, S // 2 + 32, T), U32)] * 2,
        [pltpu.VMEM((1, DH + 1, T, T), F32)] * 2,
        [pltpu.VMEM((1, NB + 1, DH // 8, 8, BQ), F32)] * 2,
        pltpu.VMEM((1, 2 * DH, T), F32),
        pltpu.VMEM((3, NB, T, BQ), F32),
        pltpu.VMEM((T, BQ), BF16),
        pltpu.VMEM((DH + 8, BQ), F32),
    )

    def ffn_phase(wo_v, wd_v, ha_s, out_v):
        wo_in = pltpu.make_async_copy(wo_hbm, wo_v, w_sem.at[2])
        wd_in = [pltpu.make_async_copy(wd_hbm.at[:, pl.ds(n * D // 2, D // 2)], wd_v.at[n], w_sem.at[3 + n])
                 for n in range(2)]
        for ref in ha_s:
            ref[7 * NF, 0:16] = jnp.zeros((16, T), BF16)

        def operands():
            return [jnp.stack(_lhs_ops(_lhs_op(i, _grid(2, lambda p, q: h_s[0, p, q, :S // 4, :])))) for i in range(7)]

        size = [jnp.sum(jnp.abs(wgu_v[0, u, 0:32, :].astype(F32)), keepdims=True) + 1e-30 for u in range(2)]
        ratio = jnp.clip(size[0] / size[1] * math.sqrt(2.0), 2.0 ** -20, 2.0 ** 20)
        ratio = pltpu.bitcast(_bits(jnp.broadcast_to(ratio, (8, T))) & 0x7F800000, F32)
        half, ratio = jnp.max(0.5 / ratio), jnp.max(ratio)

        @pl.loop(0, NF)
        def _(f):
            @pl.when(f > 0)
            def _():
                for c in gu_copies(f):
                    c.wait()

            @pl.when(f + 1 < NF)
            def _():
                for c in gu_copies(f + 1):
                    c.start()
            for k, c in enumerate(wd_in + [wo_in]):
                pl.when(f == 1 + k)(c.start)

            @pl.when(ratio != 1.0)
            def _():
                wgu_v[f & 1, 1] = (wgu_v[f & 1, 1].astype(F32) * ratio).astype(BF16)

            z1, before = z_s[1], operands()

            def job(i, r):
                ha_s[i][pl.ds(7 * f, 7), r:r + 16, :] = before[i][:, r:r + 16].astype(BF16)
                return _words(ha_s[i], 7 * NF + z1, slice(0, 8))

            def emit(r, c, v):
                h_s[0, r, c, :S // 4] = (jnp.tanh(0.5 * v[:, :T]) * half + half) * v[:, T:]
            _matmul_hk(xb, lambda r, c, u: wgu_v[f & 1, u, r * D // 4:(r + 1) * D // 4, c * T:(c + 1) * T],
                       emit, t2_s, inner,
                       _spread(([lambda i=i, r=r: job(i, r) for r in range(0, S // 4, 16) for i in range(7)], 68)))

        wo_in.wait()
        z0, z1, last = z_s[0], z_s[1], operands()

        def last_job(part, r):
            for i in part:
                xb_s[i][pl.ds(z0, 7), r // (2 * T), r % (2 * T):r % (2 * T) + 16] = last[i][:, r:r + 16].astype(BF16)
            return _tree([_words(xb_s[i], 7 + z1, 0, slice(0, 8)) for i in part], jnp.bitwise_or)

        def emit_s(r, c, v):
            for b in range(NB):
                out_v[b // 2, c // 2, (b % 2) * BQ + r * T:(b % 2) * BQ + (r + 1) * T,
                      (c % 2) * 2 * T:(c % 2 + 1) * 2 * T] = v[b * T:(b + 1) * T].astype(BF16)
        ops = _lhs_ops(_grid(2, lambda r, c: h_s[1, r, c, :S // 4, :]))
        _matmul(lambda i: (_words(ha_s[i // 7], i % 7), ops[i].astype(BF16)),
                lambda r, c: wo_v[r * D // 4:(r + 1) * D // 4, c * D // 4:(c + 1) * D // 4], emit_s, [outer, inner],
                _spread(*[([lambda p=p, r=r: last_job(p, r) for r in range(0, S // 4, 16)], 7)
                          for p in ((1, 5), (3,), (4, 6), (2,), (0,))]))

        def out_copies(it, last):
            hb, hc = BQ // 2, D // 4
            parts = [(b * BQ + hb, hc, hc) for b in range(2)] if last else (
                [(b * BQ, 0, 2 * hc) for b in range(2)] + [(b * BQ + hb, 0, hc) for b in range(2)])
            return [pltpu.make_async_copy(
                out_v.at[it >> 1, it & 1, pl.ds(r, hb), pl.ds(c, w)],
                out_hbm.at[pl.ds(pl.multiple_of((it >> 1) * (S // 2) + r, hb), hb),
                           pl.ds(pl.multiple_of((it & 1) * (D // 2) + c, hc), w)],
                out_sem) for r, c, w in parts]

        for c in wd_in:
            c.wait()

        @pl.loop(0, 4)
        def _(it):
            m, n = it >> 1, it & 1
            rows = pl.ds(pl.multiple_of(m * T, T), T)

            def emit(r, c, y):
                g = y * (0.5 * jnp.tanh(0.5 * y) + 0.5)
                for b in range(2):
                    ix = (m, n, slice(b * BQ + r * T, b * BQ + (r + 1) * T), slice(c * T, (c + 1) * T))
                    x = x_v[2 * m + b, r * T:(r + 1) * T, pl.ds(pl.multiple_of((4 * n + c) * T, T), T)]
                    out_v[ix] = (x.astype(F32) + out_v[ix].astype(F32) * g[b * T:(b + 1) * T]).astype(BF16)
                if (r, c) == (1, 1):
                    for cp in out_copies(it, False):
                        cp.start()
            _matmul(lambda i: (jnp.concatenate([_words(ha_s[i // 7], 7 * f + i % 7, rows) for f in range(1, NF)]
                                               + [_words(xb_s[i // 7], i % 7, m)], axis=1),),
                    lambda r, c: jnp.concatenate(
                        [wd_v[n, (4 * f + r) * T:(4 * f + r + 1) * T, c * T:(c + 1) * T] for f in range(NF)], axis=0),
                    emit, [lambda: [None] * 5] * 2, _spread())
            for cp in out_copies(it, True):
                cp.start()

        for it in range(4):
            for cp in out_copies(it, False) + out_copies(it, True):
                cp.wait()

    pl.run_scoped(
        ffn_phase,
        pltpu.VMEM((D, D), BF16),
        pltpu.VMEM((2, F, D // 2), BF16),
        [pltpu.VMEM((7 * NF + 1, S // 4, T), BF16)] * 7,
        pltpu.VMEM((2, 2, S // 2, D // 2), BF16),
    )


@jax.jit
def pallas_recurrent_scan__softmax_full_mha__glu_gated_glu__prompt_kernel(
    A_x: jax.Array,
    A_wqkv: jax.Array,
    A_wo: jax.Array,
    B_x: jax.Array,
    B_w_gate: jax.Array,
    B_w_up: jax.Array,
    B_w_down: jax.Array,
):
    del B_x
    in_hbm = pl.BlockSpec(memory_space=pl.ANY)
    out = pl.pallas_call(
        _kernel,
        out_shape=jax.ShapeDtypeStruct((S, D), BF16),
        in_specs=[in_hbm] * 6,
        out_specs=in_hbm,
        scratch_shapes=[
            pltpu.VMEM((NB, BQ, D), BF16),
            pltpu.VMEM((2, 2, D, 4 * T), BF16),
            [pltpu.VMEM((8, 2, S // 8, T), BF16)] * len(HK),
            pltpu.VMEM((2, 4, 4, S // 4 + 32, T), F32),
            [pltpu.VMEM((S // 4, D // 4), F32)] * 10,
            [pltpu.VMEM((S // 4, D // 4), F32)] * 20,
            pltpu.SMEM((16,), jnp.int32),
            pltpu.SemaphoreType.DMA((2 * NB,)),
            pltpu.SemaphoreType.DMA((NG // 2,)),
            pltpu.SemaphoreType.DMA((5,)),
            pltpu.SemaphoreType.DMA((2, 2)),
            pltpu.SemaphoreType.DMA(()),
        ],
        compiler_params=pltpu.CompilerParams(vmem_limit_bytes=126 * 2 ** 20, disable_bounds_checks=True),
        name="fused_block",
    )(A_x.reshape(S, D), A_wqkv, A_wo, B_w_gate, B_w_up, B_w_down)
    return out.reshape(A_x.shape)
```

```python
import math

import jax
import jax.numpy as jnp
import numpy as np
from jax import lax
import jax.experimental.pallas as pl
import jax.experimental.pallas.tpu as pltpu

F32 = jnp.float32
BF16 = jnp.bfloat16
U32 = jnp.uint32

S, D, F, H = 2048, 1024, 3584, 32
DH = D // H
T = 128
BQ = 512
NB = S // BQ
NG = D // T
NC = S // T
NF = F // (4 * T)
NV = 16
KB = 2
QSCALE = DH ** -0.5 * math.log2(math.e)
SUM_RANGE = 2.0 ** 60


def _dot(a, b):
    return jnp.dot(a, b, preferred_element_type=F32)


def _bits(v):
    return pltpu.bitcast(v, U32)


def _tree(xs, op):
    xs = list(xs)
    while len(xs) > 1:
        xs = [op(xs[i], xs[i + 1]) if i + 1 < len(xs) else xs[i] for i in range(0, len(xs), 2)]
    return xs[0]


def _tie(w, zeros):
    if not zeros:
        return w
    n = w.shape[0] // 8
    at = {((u + 1) * n) // len(zeros) - 1: _bits(z) for u, z in enumerate(zeros)}
    head = jnp.concatenate([w[8 * r:8 * r + 8, :T] | at[r] if r in at else w[8 * r:8 * r + 8, :T]
                            for r in range(n)], axis=0)
    return jnp.concatenate([head, w[:, T:]], axis=1) if w.shape[1] > T else head


def _spread(*phases):
    for jobs, steps in phases:
        for k in range(steps):
            yield [job() for job in jobs[k * len(jobs) // steps:(k + 1) * len(jobs) // steps]]
    while True:
        yield []


def _shares(jobs, weights):
    cuts = [len(jobs) * sum(weights[:i]) // sum(weights) for i in range(len(weights) + 1)]
    return [(jobs[lo:hi], 7) for lo, hi in zip(cuts, cuts[1:])]


def _force(g):
    return g() if callable(g) else g


def _add(p, q):
    if isinstance(p, tuple):
        return tuple(_add(a, b) for a, b in zip(p, q))
    return _force(p).astype(F32) + _force(q).astype(F32)


def _sub(p, q):
    if isinstance(p, tuple):
        return tuple(_sub(a, b) for a, b in zip(p, q))
    return _force(p).astype(F32) - _force(q).astype(F32)


def _grid(levels, block, r=0, c=0):
    if levels == 0:
        return lambda: block(r, c)
    return tuple(tuple(_grid(levels - 1, block, 2 * r + i, 2 * c + j) for j in range(2)) for i in range(2))


def _leaves(g, r=0, c=0):
    if isinstance(g, tuple):
        for i in range(2):
            for j in range(2):
                yield from _leaves(g[i][j], 2 * r + i, 2 * c + j)
    else:
        yield r, c, g


def _park(refs, g):
    if refs is None:
        return g
    if isinstance(g, tuple):
        return tuple(tuple(_park(refs[2 * r + c], g[r][c]) for c in range(2)) for r in range(2))
    ix = (slice(0, g.shape[0]), slice(0, g.shape[1]))
    refs[ix] = g
    return lambda: refs[ix]


def _lhs_op(i, a):
    (a11, a12), (a21, a22) = a
    if i in (2, 3):
        return a11 if i == 2 else a22
    op, p, q = {0: (_add, a11, a22), 1: (_add, a21, a22), 4: (_add, a11, a12),
                5: (_sub, a21, a11), 6: (_sub, a12, a22)}[i]
    return op(p, q)


def _rhs_op(i, b):
    (b11, b12), (b21, b22) = b
    if i in (1, 4):
        return b11 if i == 1 else b22
    op, p, q = {0: (_add, b11, b22), 2: (_sub, b12, b22), 3: (_sub, b21, b11),
                5: (_add, b11, b12), 6: (_add, b21, b22)}[i]
    return op(p, q)


def _lhs_ops(a):
    if not isinstance(a, tuple):
        return [_force(a)]
    return [op for i in range(7) for op in _lhs_ops(_lhs_op(i, a))]


def _strassen(lhs, b, emit, tmp, side, idx=0):
    def m(i):
        rhs = _rhs_op(i, b)
        if isinstance(rhs, tuple):
            c = {}
            _strassen(lhs, rhs, lambda r, s, v: c.update({(r, s): v}), tmp[1:], side, 7 * idx + i)
            return ((c[0, 0], c[0, 1]), (c[1, 0], c[1, 1]))
        a, *more = lhs(7 * idx + i)
        a = pltpu.bitcast(_tie(a, next(side)), BF16)
        return _dot(jnp.concatenate([a] + more, axis=1) if more else a, _force(rhs).astype(BF16))
    t = tmp[0]()
    m2 = _park(t[0], m(1))
    m4 = m(3)
    emit(1, 0, _add(m2, m4))
    m4 = _park(t[1], m4)
    m5 = _park(t[2], m(4))
    m3 = m(2)
    emit(0, 1, _add(m3, m5))
    t22 = _park(t[3], _sub(m3, m2))
    m1 = _park(t[4], m(0))
    emit(0, 0, _add(_sub(_add(m(6), m1), m5), m4))
    emit(1, 1, _add(_add(m(5), m1), t22))


def _matmul(lhs, w, emit, tmp, side):
    def emit_grid(i, j, g):
        for r, c, v in _leaves(g, i, j):
            emit(r, c, v)
    _strassen(lhs, _grid(len(tmp), w), emit_grid, tmp, side)


def _hopcroft_kerr():
    u = np.array([[1, 0], [0, 1], [-1, -1]])
    v = np.array([[0, -1], [1, 0], [-1, 1]])
    e = np.eye(4, dtype=int)
    kind = (1, 0, 2, 1)
    prods = []

    def inner(r, c, p, q):
        prods.extend([(np.outer(r, u[p]), np.outer(c, v[q])), (np.outer(r, u[q]), np.outer(c, v[p]))])

    def pair(ra, ca, s, rb, cb, t):
        prods.append((np.outer(ra, u[t]) + np.outer(rb, u[s]), np.outer(ca, v[t]) - np.outer(cb, v[s])))
        inner(rb - ra, cb + ca, t, s)
    for i in range(4):
        inner(e[i], e[i], (kind[i] + 1) % 3, (kind[i] + 2) % 3)
    for i, j in ((0, 1), (0, 2), (1, 2), (1, 3), (2, 3)):
        pair(e[i], e[i], kind[i], e[j], e[j], kind[j])
    pair(e[1] - e[0], e[1] + e[0], 2, e[3], e[3], kind[3])
    return prods


HK = _hopcroft_kerr()
HK_ORDER = (4, 8, 0, 11, 3, 14, 6, 20, 17, 23, 2, 10, 1, 9, 7, 19, 18, 25, 5, 24, 13, 12, 15, 16, 22, 21)


def _hk_operand(coef, block):
    pos = [block(i, k) for (i, k), c in np.ndenumerate(coef) if c > 0]
    neg = [block(i, k) for (i, k), c in np.ndenumerate(coef) if c < 0]
    if not pos:
        return -1, _tree(neg, _add)
    return 1, _sub(_tree(pos, _add), _tree(neg, _add)) if neg else _tree(pos, _add)


def _matmul_hk(lhs, w, emit, slots, inner, side):
    slots = iter(slots)

    def m(i):
        sign, rhs = _hk_operand(HK[i][1], lambda c, k: _grid(1, lambda q, u: w(2 * k + q, c, u)))
        c = {}
        _strassen(lhs, rhs, lambda r, s, v: c.update({(r, s): v}), [inner], side, i)
        v = jnp.concatenate([jnp.concatenate([c[r, 0], c[r, 1]], axis=1) for r in range(2)], axis=0)
        return sign * (1 if (HK[i][0] > 0).any() else -1), v

    def park(sign, v):
        return sign, _park(next(slots), v)

    def total(*terms):
        sign, v = terms[0][0] * terms[0][1][0], terms[0][1][1]
        for k, (s, g) in terms[1:]:
            if k * s == sign:
                v = _add(v, g)
            elif sign > 0:
                v = _sub(v, g)
            else:
                sign, v = 1, _sub(g, v)
        return sign, v

    def out(r, c, *terms):
        sign, v = total(*terms)
        emit(r, c, v if sign > 0 else -v)
        return sign, v

    def diagonal(k):
        v = m(k)
        out(k // 2, k // 2, (1 - 2 * (k % 2), v), (2 * (k % 2) - 1, p[k ^ 1]))
        p[k] = park(*v)

    p = {i: park(*m(i)) for i in HK_ORDER[:10]}
    diagonal(2)
    p10 = m(10)
    out(0, 1, (1, p10), (-1, p[8]), (-1, p[0]), (1, p[2]))
    p10 = park(*p10)
    diagonal(1)
    p9 = m(9)
    out(1, 0, (1, p9), (-1, p[8]), (-1, p[1]), (1, p[3]))
    p9 = park(*p9)
    diagonal(7)
    y13 = out(1, 3, (-1, m(19)), (1, p[17]), (1, p[3]), (-1, p[7]))
    t03 = park(*total((1, y13), (-1, p[6]), (1, p9)))
    y31 = out(3, 1, (-1, m(18)), (1, p[17]), (1, p[2]), (-1, p[6]))
    t30 = park(*total((-1, y31), (1, p[7]), (-1, p10)))
    out(0, 3, (-1, m(25)), (1, p[23]), (1, t03))
    diagonal(5)
    out(3, 0, (1, m(24)), (-1, p[23]), (1, t30))
    out(0, 2, (-1, m(13)), (1, p[11]), (1, p[1]), (-1, p[5]))
    out(2, 0, (-1, m(12)), (1, p[11]), (1, p[0]), (-1, p[4]))
    out(2, 1, (1, m(15)), (-1, p[14]), (-1, p[3]), (1, p[5]))
    out(1, 2, (1, m(16)), (-1, p[14]), (-1, p[2]), (1, p[4]))
    out(2, 3, (1, m(22)), (-1, p[20]), (-1, p[4]), (1, p[6]))
    out(3, 2, (1, m(21)), (-1, p[20]), (-1, p[5]), (1, p[7]))


def _kernel(x_hbm, wqkv_hbm, wo_hbm, wg_hbm, wu_hbm, wd_hbm, out_hbm,
            x_v, wgu_v, xb_s, h_s, t1_s, t2_s, z_s, x_sem, wk_sem, w_sem, gu_sem, out_sem):
    turn = [0]

    def inner():
        turn[0] ^= 5
        return t1_s[turn[0]:turn[0] + 5]

    def outer():
        return [t2_s[4 * k:4 * k + 4] for k in range(5)]

    def xb(i):
        return jnp.concatenate([xb_s[i // 7][t, :, i % 7 * T:(i % 7 + 1) * T] for t in range(2)], axis=1),

    def gu_copies(f):
        cols = pl.ds(pl.multiple_of(f * 4 * T, 4 * T), 4 * T)
        return [pltpu.make_async_copy(w.at[:, cols], wgu_v.at[f & 1, j], gu_sem.at[f & 1, j])
                for j, w in enumerate((wg_hbm, wu_hbm))]

    def attention_phase(wk_v, wqv_v, xn_s, xa_s, k_s, q_s, v_s, kh_s, kb_s, qf_s, kv_s, ot_s, p_s, acc_s):
        n = BQ // 2
        x_in = [pltpu.make_async_copy(x_hbm.at[pl.ds(i * n, n)], x_v.at[i // 2, pl.ds(i % 2 * n, n)], x_sem.at[i])
                for i in range(2 * NB)]
        wk_in = [pltpu.make_async_copy(wqkv_hbm.at[:, pl.ds(D + j * 2 * T, 2 * T)], wk_v[j], wk_sem.at[j])
                 for j in range(NG // 2)]
        wqv_in = [pltpu.make_async_copy(wqkv_hbm.at[:, pl.ds(2 * j * D, D)], wqv_v.at[j], w_sem.at[j])
                  for j in range(2)]

        def layernorm(b, r, rows, z):
            x = x_v[b, r:r + rows, :].astype(F32)
            xc = x - jnp.mean(x, axis=-1, keepdims=True)
            xn = xc * lax.rsqrt(jnp.mean(xc * xc, axis=-1, keepdims=True) + 1e-5)
            for t in range(NG):
                xn_s[b][t + z, r:r + rows, :] = xn[:, t * T:(t + 1) * T]

        def layernorm_jobs(b):
            z0, z1 = z_s[0], z_s[1]

            def job(r):
                layernorm(b, r, 16, z0)
                return xn_s[b][NG + z1, 0:8, :]
            return [lambda r=r: job(r) for r in range(0, BQ, 16)]

        def xa(lo, hi, first):
            ops = _lhs_ops(_grid(2, lambda r, c: jnp.concatenate([jnp.concatenate(
                [xn_s[b][2 * c + t, r * T:(r + 1) * T, :] for t in range(2)], axis=1) for b in range(lo, hi)], axis=0)))

            def lhs(i):
                xa_s[i, lo * T // 2:hi * T // 2] = _bits(ops[i].astype(BF16))
                return xa_s[i, first * T // 2:],
            return lhs

        def xb_jobs(which):
            z0, z1 = z_s[0], z_s[1]

            def block(t, z):
                return lambda r, k: _grid(1, lambda u, q: jnp.concatenate(
                    [xn_s[b][z + 2 * (2 * k + q) + t, r * T:(r + 1) * T, :] for b in (2 * u, 2 * u + 1)], axis=0))
            ops = {(i, t): jnp.concatenate(_lhs_ops(_hk_operand(HK[i][0], block(t, z_s[n]))[1]), axis=1)
                   for n, i in enumerate(which) for t in range(2)}

            def job(i, row, t):
                xb_s[i][t + z0, row // 2:row // 2 + 8, :7 * T] = _bits(ops[i, t][row:row + 16].astype(BF16))
                return xb_s[i][z1, 0:8, 7 * T:]
            return [lambda i=i, row=row, t=t: job(i, row, t)
                    for row in range(0, 2 * T, 16) for t in range(2) for i in which]

        def emit_k(r, c, v):
            for b in range(KB, NB):
                for u in range(2):
                    k_s[2 * c + u, (4 * b + r) * T // 2:(4 * b + r + 1) * T // 2] = _bits(
                        v[(b - KB) * T:(b - KB + 1) * T, u * T:(u + 1) * T].astype(BF16))

        def emit_transposed(ref, r, c, v):
            for b in range(NB):
                for u in range(2):
                    heads = slice(4 * (2 * c + u), 4 * (2 * c + u + 1))
                    ref[heads, b, :, r * T:(r + 1) * T] = _bits(
                        v[b * T:(b + 1) * T, u * T:(u + 1) * T].T.astype(BF16)).reshape(4, DH // 2, T)

        def to_lane0(k, h):
            return pltpu.roll(k, (T - DH * (h & 3)) & (T - 1), 1)

        def head_jobs(h, slot, after=lambda v: v):
            z0, z1 = z_s[0], z_s[1]

            def pick():
                kv = jnp.concatenate([k_s[h >> 2, r - NV // 2:r] for r in range(T, S // 2 + 1, T)], axis=0)
                kv_s[z0, :DH] = pltpu.bitcast(to_lane0(after(kv), h), BF16).astype(F32).T[:DH]
                return kv_s[z1, DH:DH + 8]

            def queries(b):
                qf_s[slot][z0, b] = pltpu.bitcast(after(q_s[h, b]), BF16).astype(F32).reshape(DH // 8, 8, BQ)
                return qf_s[slot][z1, NB, 0, :, 0:T]

            def move(r):
                kh_s[slot][z0, r:r + T, :] = to_lane0(after(k_s[h >> 2, r:r + T]), h)
                return kh_s[slot][z1, S // 2:S // 2 + 8, :]

            def splat(d):
                kb_s[slot][z0, d] = after(jnp.broadcast_to(kv_s[0, d:d + 1, :], (T, T))).T
                return kb_s[slot][z1, DH, 0:8, :]
            return ([pick] + [lambda b=b: queries(b) for b in range(NB)]
                    + [lambda r=r: move(r) for r in range(0, S // 2, T)] + [lambda d=d: splat(d) for d in range(DH)])

        def output_jobs(g, b, after=lambda v: v):
            z1 = z_s[1]

            def job(r):
                h_s[g & 1, r, g >> 1, pl.ds(pl.multiple_of(b * T, T), T), :] = after(ot_s[g & 1, b, :, r * T:(r + 1) * T]).T
                return h_s[z1, 0, 0, S // 4:S // 4 + 8, :]
            return [lambda r=r: job(r) for r in range(4)]

        def put_head(h, b, o):
            ot_s[(h >> 2) & 1, b, pl.ds(pl.multiple_of((h & 3) * DH, DH), DH), :] = o

        def pv(ties, acc, h, b, c, p, l):
            a = _dot(pltpu.bitcast(v_s[h + z_s[b], c // 4, :, c % 4 * T:(c % 4 + 1) * T], BF16), p)
            if c > 0:
                a = acc + a
            if c == NC - 1:
                l = jnp.sum(l, axis=0, keepdims=True)
                r = pltpu.reciprocal(l, approx=True)
                r = r * (2.0 - l * r)
                o = a * r
                put_head(h, b, o)
                ot_s[2 + z_s[0], 0, 8:16, :] += _tree([o[t:t + 8] for t in range(0, DH, 8)], jnp.add) * 0.0 + (l + r)
                ties.append(ot_s[2 + z_s[1], 0, 0:8, 0:T])
            return a

        def attention(h, slot):
            acc, pend = acc_s[:DH], [((h + H - 1) & (H - 1), NB - 1, NC - 1, p_s[...], acc_s[DH:])]
            zero = jnp.tile(_bits(h_s[z_s[1], 0, 0, S // 4:S // 4 + 8, :]), (NV // 8, 1))
            now, ties = [None], []

            def after(v):
                z = jnp.tile(_bits(now[0]) & zero[:8], (1, v.shape[1] // T))
                return jnp.concatenate([pltpu.bitcast(_bits(v[:8]) | z, v.dtype), v[8:]], axis=0)

            def vector_scores(b, e):
                cols = []
                for t in range(BQ // T):
                    z = z_s[e]
                    q = jnp.stack([jnp.broadcast_to(qf_s[slot][z, b, :, i:i + 1, t * T:(t + 1) * T], (DH // 8, NV, T))
                                   for i in range(8)], axis=1).reshape(DH, NV, T)
                    v = kb_s[slot][z_s[4 * b + t], :DH, e * NV:(e + 1) * NV, :] * q
                    if cols:
                        first = pltpu.bitcast(_bits(v[0]) | (_bits(cols[-1]) & zero), F32)
                        v = jnp.concatenate([first[None], v[1:]], axis=0)
                    cols.append(jnp.sum(v, axis=0))
                return jnp.concatenate(cols, axis=1)

            side = _spread(([], 2),
                           (output_jobs(((h >> 2) + NG - 1) & (NG - 1), h & 3, after), 4),
                           (head_jobs(jnp.minimum(h + 1, H - 1), 1 - slot, after), 55))
            late = [[]] * 3
            for b in range(NB):
                l = None
                for c in range(NC):
                    nv = NV if c % 2 and (b, c) != (0, 1) else 0
                    late.append(next(side))
                    k = _tie(kh_s[slot][z_s[b], c * T // 2:((c + 1) * T - nv) // 2, :],
                             late.pop(0) + ([ties.pop()] if c == 3 else []))
                    s = _dot(pltpu.bitcast(k, BF16)[:, :DH], pltpu.bitcast(q_s[h + z_s[c], b], BF16))
                    now[0] = s[96:104, :T]
                    if nv:
                        s = jnp.concatenate([s, vector_scores(b, c // 2)], axis=0)
                    p = jnp.exp2(s)
                    for t in range(0, T, 16):
                        two = p[t:t + 8] + p[t + 8:t + 16]
                        l = two if l is None else l + two
                    pend.append((h, b, c, p.astype(BF16), l))
                    if len(pend) > 2:
                        acc = pv(ties, acc, *pend.pop(0))
            acc_s[:DH] = pv(ties, acc, *pend.pop(0))
            p_s[...], acc_s[DH:] = pend[0][3:]

        def exact_attention(job, _):
            h, b = job >> 2, job & 3
            q = pltpu.bitcast(q_s[h, b], BF16)

            def step(i, carry):
                m, l, acc = carry
                k = to_lane0(k_s[h >> 2, pl.ds(pl.multiple_of(i * (BQ // 2), BQ // 2), BQ // 2)], h)
                s = _dot(pltpu.bitcast(k, BF16)[:, :DH], q)
                top = jnp.maximum(m, jnp.max(s, axis=0, keepdims=True))
                alpha, p = jnp.exp2(m - top), jnp.exp2(s - top)
                return (top, l * alpha + jnp.sum(p, axis=0, keepdims=True),
                        acc * alpha + _dot(pltpu.bitcast(v_s[h, i], BF16), p.astype(BF16)))
            _, l, acc = lax.fori_loop(0, NB, step, (jnp.full((1, BQ), -jnp.inf, F32), jnp.zeros((1, BQ), F32),
                                                    jnp.zeros((DH, BQ), F32)))
            put_head(h, b, acc / l)

            @pl.when((h & 3) == 3)
            def _():
                for run in output_jobs(h >> 2, b):
                    run()

        for c in x_in[:2] + wk_in[:1]:
            c.start()

        @pl.loop(0, z_s.shape[0])
        def _(i):
            z_s[i] = 0
        for ref in t1_s + t2_s:
            ref[pl.ds(pl.multiple_of(z_s[0], 8), 8), 0:T] = jnp.zeros((8, T), F32)
        for ref in xn_s:
            ref[NG + z_s[0], 0:8] = jnp.zeros((8, T), F32)
        xa_s[z_s[0], 0:8, 0:T] = jnp.zeros((8, T), U32)
        for ref in xb_s:
            ref[0, 0:8, 7 * T:] = jnp.zeros((8, T), U32)
        for slot in range(2):
            kh_s[slot][0, S // 2:S // 2 + 8, :] = jnp.zeros((8, T), U32)
            qf_s[slot][0, NB, 0, :, 0:T] = jnp.zeros((8, T), F32)
            kb_s[slot][0, DH, 0:8, :] = jnp.zeros((8, T), F32)
        h_s[0, 0, 0, S // 4:S // 4 + 8, :] = jnp.zeros((8, T), F32)
        kv_s[0, DH:DH + 8] = jnp.zeros((8, T), F32)
        ot_s[1] = jnp.zeros((NB, T, BQ), F32)
        ot_s[2, 0, 0:16] = jnp.zeros((16, BQ), F32)
        p_s[...] = jnp.zeros(p_s.shape, BF16)
        acc_s[...] = jnp.ones(acc_s.shape, F32)

        for i in range(2):
            x_in[i].wait()
            wk_in[i + 1].start()
            for r in range(i * n, (i + 1) * n, 32):
                layernorm(0, r, 32, 0)
        traffic = {0: ([wk_in[0]], [x_in[2]]), 1: ([wk_in[1]], [wk_in[3], x_in[3]]),
                   2: ([wk_in[2], x_in[2]], [x_in[4]]), 3: ([wk_in[3], x_in[3]], x_in[5:7]),
                   4: (x_in[4:6], [wqv_in[0], x_in[7]]), 6: (x_in[6:8], [])}
        side = _spread()
        for step in range(KB * NG // 2):
            b, j = divmod(step, NG // 2)
            wait, start = traffic.get(step, ([], []))
            for c in wait:
                c.wait()
            for c in start:
                c.start()
            if j == 0:
                ops = [(_bits(v[:, :T].astype(BF16)), v[:, T:].astype(BF16)) for v in _lhs_ops(_grid(
                    1, lambda r, c: jnp.concatenate([xn_s[b][4 * c + t, r * n:(r + 1) * n, :] for t in range(4)], axis=1)))]
            if step == 2:
                jobs = layernorm_jobs(1)
                side = _spread(([], 1), (jobs[:16], 6), ([], 1), (jobs[16:], 6))
            if step in (4, 6):
                side = _spread(([], 1), (layernorm_jobs(step // 2), 13))

            def emit(r, c, v):
                k_s[2 * j + c, (2 * b + r) * T:(2 * b + r + 1) * T] = _bits(v.astype(BF16))
            _matmul(lambda i: ops[i], lambda r, c: wk_v[j][r * D // 2:(r + 1) * D // 2, c * T:(c + 1) * T],
                    emit, [inner], side)

        wqv_in[0].wait()
        for c in wqv_in[1:] + gu_copies(0):
            c.start()
        _matmul(xa(KB, NB, KB), lambda r, c: wk_v[c][r * D // 4:(r + 1) * D // 4, :], emit_k, [outer, inner], _spread())
        _matmul(xa(0, KB, 0), lambda r, c: wqv_v[0, r * D // 4:(r + 1) * D // 4, c * D // 4:(c + 1) * D // 4],
                lambda r, c, v: emit_transposed(q_s, r, c, v * QSCALE), [outer, inner],
                _spread(*_shares(xb_jobs(HK_ORDER[:16]), (4, 1, 5, 1, 5, 1, 1))))
        wqv_in[1].wait()
        _matmul_hk(xb, lambda r, c, u: wqv_v[1, r * D // 4:(r + 1) * D // 4, (2 * c + u) * T:(2 * c + u + 1) * T],
                   lambda r, c, v: emit_transposed(v_s, r, c, v), t2_s, inner,
                   _spread((xb_jobs(HK_ORDER[16:]), 70), (head_jobs(0, 0), 100)))
        for c in gu_copies(0):
            c.wait()

        @pl.loop(0, H // 2)
        def _(i):
            attention(2 * i, 0)
            pl.when(z_s[0] == 0)(lambda: attention(2 * i + 1, 1))

        size = [jnp.sum(sum(jnp.abs(wgu_v[0, u, r:r + 16, :].astype(F32)) for r in range(0, D, D // 4)), keepdims=True)
                for u in range(2)]
        ratio = size[0] / size[1] * math.sqrt(2.0)
        ratio = jnp.where((ratio > 2.0 ** -20) & (ratio < 2.0 ** 20), ratio, 1.0)
        ratio = pltpu.bitcast(_bits(jnp.broadcast_to(ratio, (8, T))) & 0x7F800000, F32)
        half, ratio = jnp.max(0.5 / ratio), jnp.max(ratio)

        for b in range(NB):
            if b == NB - 1:
                pv([], acc_s[:DH], H - 1, b, NC - 1, p_s[...], acc_s[DH:])
            for run in output_jobs(NG - 1, b):
                run()

        @pl.when(jnp.max(jnp.where(jnp.abs(ot_s[2, 0, 8:16, :]) <= SUM_RANGE, 0, 1)) > 0)
        def _():
            lax.fori_loop(0, H * NB, exact_attention, None)
        return half, ratio

    half, ratio = pl.run_scoped(
        attention_phase,
        [pltpu.VMEM((D, 2 * T), BF16)] * (NG // 2),
        pltpu.VMEM((2, D, D), BF16),
        [pltpu.VMEM((NG + 1, BQ, T), F32)] * NB,
        pltpu.VMEM((49, S // 8, 2 * T), U32),
        pltpu.VMEM((NG, S // 2, T), U32),
        pltpu.VMEM((H, NB, DH // 2, BQ), U32),
        pltpu.VMEM((H, NB, DH // 2, BQ), U32),
        [pltpu.VMEM((1, S // 2 + 32, T), U32)] * 2,
        [pltpu.VMEM((1, DH + 1, T, T), F32)] * 2,
        [pltpu.VMEM((1, NB + 1, DH // 8, 8, BQ), F32)] * 2,
        pltpu.VMEM((1, 2 * DH, T), F32),
        pltpu.VMEM((3, NB, T, BQ), F32),
        pltpu.VMEM((T, BQ), BF16),
        pltpu.VMEM((DH + 8, BQ), F32),
    )

    def ffn_phase(wo_v, wd_v, ha_s, out_v):
        wo_in = pltpu.make_async_copy(wo_hbm, wo_v, w_sem.at[2])
        wd_in = [pltpu.make_async_copy(wd_hbm.at[:, pl.ds(n * D // 2, D // 2)], wd_v.at[n], w_sem.at[3 + n])
                 for n in range(2)]
        for ref in ha_s:
            ref[0, S // 8:S // 8 + 8, 0:T] = jnp.zeros((8, T), U32)

        def operands():
            return [jnp.concatenate(_lhs_ops(_lhs_op(i, _grid(2, lambda p, q: h_s[0, p, q, :S // 4, :]))), axis=1)
                    for i in range(7)]

        @pl.loop(0, NF)
        def _(f):
            @pl.when(f > 0)
            def _():
                for c in gu_copies(f):
                    c.wait()

            @pl.when(f + 1 < NF)
            def _():
                for c in gu_copies(f + 1):
                    c.start()
            for k, c in enumerate(wd_in + [wo_in]):
                pl.when(f == 1 + k)(c.start)

            @pl.when(ratio != 1.0)
            def _():
                wgu_v[f & 1, 1] = (wgu_v[f & 1, 1].astype(F32) * ratio).astype(BF16)

            z1, before = z_s[1], operands()

            def job(i, r):
                ha_s[i][f, r // 2:r // 2 + 8] = _bits(before[i][r:r + 16].astype(BF16))
                return ha_s[i][z1, S // 8:S // 8 + 8, 0:T]

            def emit(r, c, v):
                h_s[0, r, c, :S // 4] = (jnp.tanh(0.5 * v[:, :T]) * half + half) * v[:, T:]
            _matmul_hk(xb, lambda r, c, u: wgu_v[f & 1, u, r * D // 4:(r + 1) * D // 4, c * T:(c + 1) * T],
                       emit, t2_s, inner,
                       _spread(*_shares([lambda i=i, r=r: job(i, r) for r in range(0, S // 4, 16) for i in range(7)],
                                        (4, 3, 4, 3, 4, 3, 4, 3, 3, 3))))

        wo_in.wait()
        z0, z1, last = z_s[0], z_s[1], operands()

        def last_job(i, r):
            xb_s[i][z0 + r // (2 * T), r // 2 % T:r // 2 % T + 8, :7 * T] = _bits(last[i][r:r + 16].astype(BF16))
            return xb_s[i][z1, 0:8, 7 * T:]

        def emit_s(r, c, v):
            for b in range(NB):
                out_v[b // 2, c // 2, (b % 2) * BQ + r * T:(b % 2) * BQ + (r + 1) * T,
                      (c % 2) * 2 * T:(c % 2 + 1) * 2 * T] = v[b * T:(b + 1) * T].astype(BF16)
        ops = _lhs_ops(_grid(2, lambda r, c: h_s[1, r, c, :S // 4, :]))
        _matmul(lambda i: (ha_s[i // 7][0, :S // 8, i % 7 * T:(i % 7 + 1) * T], ops[i].astype(BF16)),
                lambda r, c: wo_v[r * D // 4:(r + 1) * D // 4, c * D // 4:(c + 1) * D // 4], emit_s, [outer, inner],
                _spread(*_shares([lambda i=i, r=r: last_job(i, r) for r in range(0, S // 4, 16) for i in range(7)],
                                 (2, 1, 2, 1, 2))))

        def out_copies(it, last):
            hb, hc = BQ // 2, D // 4
            parts = [(b * BQ + hb, hc, hc) for b in range(2)] if last else (
                [(b * BQ, 0, 2 * hc) for b in range(2)] + [(b * BQ + hb, 0, hc) for b in range(2)])
            return [pltpu.make_async_copy(
                out_v.at[it >> 1, it & 1, pl.ds(r, hb), pl.ds(c, w)],
                out_hbm.at[pl.ds(pl.multiple_of((it >> 1) * (S // 2) + r, hb), hb),
                           pl.ds(pl.multiple_of((it & 1) * (D // 2) + c, hc), w)],
                out_sem) for r, c, w in parts]

        for c in wd_in:
            c.wait()

        @pl.loop(0, 4)
        def _(it):
            m, n = it >> 1, it & 1
            rows = pl.ds(pl.multiple_of(m * T, T), T)

            def emit(r, c, y):
                g = y * (0.5 * jnp.tanh(0.5 * y) + 0.5)
                for b in range(2):
                    ix = (m, n, slice(b * BQ + r * T, b * BQ + (r + 1) * T), slice(c * T, (c + 1) * T))
                    x = x_v[2 * m + b, r * T:(r + 1) * T, pl.ds(pl.multiple_of((4 * n + c) * T, T), T)]
                    out_v[ix] = (x.astype(F32) + out_v[ix].astype(F32) * g[b * T:(b + 1) * T]).astype(BF16)
                if (r, c) == (1, 1):
                    for cp in out_copies(it, False):
                        cp.start()
            _matmul(lambda i: (jnp.concatenate([ha_s[i // 7][f, rows, i % 7 * T:(i % 7 + 1) * T] for f in range(1, NF)]
                                               + [xb_s[i // 7][m, :, i % 7 * T:(i % 7 + 1) * T]], axis=1),),
                    lambda r, c: jnp.concatenate(
                        [wd_v[n, (4 * f + r) * T:(4 * f + r + 1) * T, c * T:(c + 1) * T] for f in range(NF)], axis=0),
                    emit, [lambda: [None] * 5] * 2, _spread())
            for cp in out_copies(it, True):
                cp.start()

        for it in range(4):
            for cp in out_copies(it, False) + out_copies(it, True):
                cp.wait()

    pl.run_scoped(
        ffn_phase,
        pltpu.VMEM((D, D), BF16),
        pltpu.VMEM((2, F, D // 2), BF16),
        [pltpu.VMEM((NF, S // 8 + 32, 7 * T), U32)] * 7,
        pltpu.VMEM((2, 2, S // 2, D // 2), BF16),
    )


@jax.jit
def pallas_recurrent_scan__softmax_full_mha__glu_gated_glu__prompt_kernel(
    A_x: jax.Array,
    A_wqkv: jax.Array,
    A_wo: jax.Array,
    B_x: jax.Array,
    B_w_gate: jax.Array,
    B_w_up: jax.Array,
    B_w_down: jax.Array,
):
    del B_x
    in_hbm = pl.BlockSpec(memory_space=pl.ANY)
    out = pl.pallas_call(
        _kernel,
        out_shape=jax.ShapeDtypeStruct((S, D), BF16),
        in_specs=[in_hbm] * 6,
        out_specs=in_hbm,
        scratch_shapes=[
            pltpu.VMEM((NB, BQ, D), BF16),
            pltpu.VMEM((2, 2, D, 4 * T), BF16),
            [pltpu.VMEM((2, S // 16, 8 * T), U32)] * len(HK),
            pltpu.VMEM((2, 4, 4, S // 4 + 32, T), F32),
            [pltpu.VMEM((S // 4, D // 4), F32)] * 10,
            [pltpu.VMEM((S // 4, D // 4), F32)] * 20,
            pltpu.SMEM((16,), jnp.int32),
            pltpu.SemaphoreType.DMA((2 * NB,)),
            pltpu.SemaphoreType.DMA((NG // 2,)),
            pltpu.SemaphoreType.DMA((5,)),
            pltpu.SemaphoreType.DMA((2, 2)),
            pltpu.SemaphoreType.DMA(()),
        ],
        compiler_params=pltpu.CompilerParams(vmem_limit_bytes=126 * 2 ** 20, disable_bounds_checks=True),
        name="fused_block",
    )(A_x.reshape(S, D), A_wqkv, A_wo, B_w_gate, B_w_up, B_w_down)
    return out.reshape(A_x.shape)
```
